```python
import jax
import jax.numpy as jnp

def _softmax(x, axis=-1):
    return jax.nn.softmax(x, axis=axis)
def _gelu(x):
    return jax.nn.gelu(x, approximate=True)
def _silu(x):
    return jax.nn.silu(x)
def _sigmoid(x):
    return jax.nn.sigmoid(x)
def _layernorm(x, axis=-1, eps=1e-5):
    m = jnp.mean(x, axis=axis, keepdims=True)
    v = jnp.var(x, axis=axis, keepdims=True)
    return (x - m) / jnp.sqrt(v + eps)
def _scatter_add(tgt, idx, src, axis=0):
    return tgt.at[idx].add(src)
def _segment_sum(src, seg, n):
    return jax.ops.segment_sum(src, seg, n)
class _Rng:
    def __init__(self, key):
        self._k = key
    def _next(self):
        self._k, sub = jax.random.split(self._k)
        return sub
    def normal(self, shape):
        return jax.random.normal(self._next(), shape, dtype=jnp.bfloat16)
    def randint(self, lo, hi, shape):
        return jax.random.randint(self._next(), shape, lo, hi, dtype=jnp.int32)
    def uniform(self, shape, lo=0.0, hi=1.0):
        return jax.random.uniform(self._next(), shape, jnp.bfloat16, lo, hi)
    def permutation(self, n):
        return jax.random.permutation(self._next(), n)


kernel_name = 'recurrent_scan__sliding_local_dilated__swiglu_ffn__prompt'

def setup_inputs():
    _rng = _Rng(jax.random.key(int.from_bytes(__import__("os").urandom(4), "little")))
    _w = (lambda a: (lambda t: t.astype(jnp.bfloat16) if jnp.issubdtype(t.dtype, jnp.floating) else t)(jnp.asarray(a)))
    def _A_setup():
        B, S, D = 1, 2048, 1024
        return {
            "x": _w((lambda *s: _rng.normal(s) * 0.05)(B, S, D)),
            "wqkv": _w((lambda *s: _rng.normal(s) * 0.05)(D, 3 * D)),
            "wo": _w((lambda *s: _rng.normal(s) * 0.05)(D, D)),
        }
    _A_in = _A_setup()

    def _B_setup():
        B, S, D, F = 1, 2048, 1024, 3584
        return {
            "x": _w((lambda *s: _rng.normal(s) * 0.05)(B, S, D)),
            "w_gate": _w((lambda *s: _rng.normal(s) * 0.05)(D, F)),
            "w_up": _w((lambda *s: _rng.normal(s) * 0.05)(D, F)),
            "w_down": _w((lambda *s: _rng.normal(s) * 0.05)(F, D)),
        }
    _B_in = _B_setup()

    return {
        "A_x": _A_in["x"],
        "A_wqkv": _A_in["wqkv"],
        "A_wo": _A_in["wo"],
        "B_x": _B_in["x"],
        "B_w_gate": _B_in["w_gate"],
        "B_w_up": _B_in["w_up"],
        "B_w_down": _B_in["w_down"],
    }

def reference(A_x, A_wqkv, A_wo, B_x, B_w_gate, B_w_up, B_w_down):
    def _A_ref(x, wqkv, wo):
        B, S, D = x.shape
        H = 32; Dh = D // H
        W, dil = 8, 2
        qkv = (lambda x, *d: x.transpose(*d))((x @ wqkv).reshape(B, S, 3, H, Dh), 2, 0, 3, 1, 4)
        q, k, v = qkv[0], qkv[1], qkv[2]
        scale = Dh ** -0.5
        pos = jnp.arange(S)
        off = jnp.arange(W) * dil
        idx = pos[:, None] - off[None, :]
        mask = idx >= 0
        idx_c = jnp.where(mask, idx, 0).reshape(-1)
        kg = k[:, :, idx_c, :].reshape(B, H, S, W, Dh)
        vg = v[:, :, idx_c, :].reshape(B, H, S, W, Dh)
        logits = jnp.einsum("bhsd,bhswd->bhsw", q, kg) * scale
        logits = jnp.where(mask[None, None, :, :], logits, -1e9)
        attn = _softmax(logits, axis=-1)
        o = jnp.einsum("bhsw,bhswd->bhsd", attn, vg)
        return (lambda x, *d: x.transpose(*d))(o, 0, 2, 1, 3).reshape(B, S, D) @ wo

    def _B_ref(x, w_gate, w_up, w_down):
        g = _silu(x @ w_gate)
        u = x @ w_up
        return (g * u) @ w_down

    x = A_x
    xn = _layernorm(x, axis=-1)
    s = _A_ref(xn, A_wqkv, A_wo)
    g = _silu(_B_ref(xn, B_w_gate, B_w_up, B_w_down))
    return x + s * g
```

```python
import functools
import math

import jax
import jax.numpy as jnp
import numpy as np
from jax import lax
from jax.experimental import pallas as pl
from jax.experimental.pallas import tpu as pltpu

S, D, F = 2048, 1024, 3584
H, DH, WIN, DIL = 32, 32, 8, 2
EPS = 1e-5
HALO = 16
bf16, f32, u32 = jnp.bfloat16, jnp.float32, jnp.uint32
NEG = -1e9


def _roll(x, s):
    return pltpu.roll(x, s % 128, 1)


def _lanebit_clear(shape, bit):
    return (lax.broadcasted_iota(jnp.int32, shape, 1) & bit) == 0


def make_kernel(SB=256, FC=512, R=8, order="qkv_first"):
    nS = S // SB
    nF = F // FC
    WOP = 65

    def kernel(x_ref, wqkv_hbm, wo_hbm, wg_hbm, wu_hbm, wd_hbm, out_ref,
               wqkv_v, wo_v, wg_v, wu_v, wd_v, wp, wop, q_s, k_s, v_s, sems):
        step = pl.program_id(0)

        def cp_qkv():
            return pltpu.make_async_copy(wqkv_hbm, wqkv_v, sems.at[0])

        def cp_wo():
            return pltpu.make_async_copy(wo_hbm, wo_v, sems.at[1])

        def cp_g(f):
            return pltpu.make_async_copy(wg_hbm.at[:, pl.ds(f * FC, FC)], wg_v.at[:, pl.ds(f * FC, FC)], sems.at[2 + 3 * f])

        def cp_u(f):
            return pltpu.make_async_copy(wu_hbm.at[:, pl.ds(f * FC, FC)], wu_v.at[:, pl.ds(f * FC, FC)], sems.at[3 + 3 * f])

        def cp_d(f):
            return pltpu.make_async_copy(wd_hbm.at[pl.ds(f * FC, FC), :], wd_v.at[pl.ds(f * FC, FC), :], sems.at[4 + 3 * f])

        def once(fn):
            pl.when(step == 0)(fn)

        @once
        def _start():
            cp_qkv().start()
            for f in range(nF):
                cp_g(f).start()
                cp_u(f).start()
                cp_d(f).start()
                if f == 1:
                    cp_wo().start()
            z = jnp.zeros((8, HALO, 128), f32)
            k_s[:, 0:HALO, :] = z
            v_s[:, 0:HALO, :] = z

        x = x_ref[...].astype(f32)
        mean = jnp.mean(x, axis=-1, keepdims=True)
        xc = x - mean
        var = jnp.mean(xc * xc, axis=-1, keepdims=True)
        xn = (xc * lax.rsqrt(var + EPS)).astype(bf16)

        def prep_qkv():
            cp_qkv().wait()
            RK = 128

            def body(it, c):
                k0 = pl.multiple_of(it * RK, RK)
                p0 = pl.multiple_of(it * (RK // 2), RK // 2)
                for m in range(3):
                    t = [pltpu.bitcast(wqkv_v[pl.ds(k0, RK), m * 1024 + 128 * j:m * 1024 + 128 * (j + 1)], u32)
                         for j in range(8)]
                    for tb, lb in ((1, 2), (2, 4), (4, 8)):
                        msk = _lanebit_clear(t[0].shape, lb)
                        n = [None] * 8
                        for a in range(8):
                            if a & tb:
                                continue
                            b = a | tb
                            n[a] = jnp.where(msk, t[a], _roll(t[b], lb))
                            n[b] = jnp.where(msk, _roll(t[a], -lb), t[b])
                        t = n
                    for j in range(8):
                        wp[pl.ds(p0, RK // 2), m * 1024 + 128 * j:m * 1024 + 128 * (j + 1)] = t[j]
                return c

            lax.fori_loop(0, D // RK, body, 0)

        def prep_wo():
            cp_wo().wait()
            for ct in range(8):
                for T in range(8):
                    blk = pltpu.bitcast(wo_v[128 * T:128 * (T + 1), 128 * ct:128 * (ct + 1)], u32)
                    for c in range(8):
                        wop[ct, pl.ds(8 * c + T, 8, stride=WOP), :] = blk[8 * c:8 * c + 8, :]

        def qkv_proj():
            for m, dst, r0 in ((0, q_s, 0), (1, k_s, HALO), (2, v_s, HALO)):
                for half in range(2):
                    c0 = m * 1024 + half * 512
                    w = pltpu.bitcast(wp[:, c0:c0 + 512], bf16)
                    y = jnp.dot(xn, w, preferred_element_type=f32)
                    for jj in range(4):
                        dst[half * 4 + jj, r0:r0 + SB, :] = y[:, 128 * jj:128 * (jj + 1)]

        shp = (R, 128)
        m16 = _lanebit_clear(shp, 16)
        m1 = _lanebit_clear(shp, 1)
        CEXP = (DH ** -0.5) * math.log2(math.e)

        def swap(z, msk, s):
            return jnp.where(msk, _roll(z, -s), _roll(z, s))

        def merge(a, b, msk, s):
            return jnp.where(msk, a + _roll(a, -s), b + _roll(b, s))

        def tree_sum(ts):
            while len(ts) > 1:
                ts = [ts[i] + ts[i + 1] for i in range(0, len(ts), 2)]
            return ts[0]

        def attn_rows(r0):
            q = [q_s[j, r0:r0 + R, :] for j in range(8)]
            P = []
            for w in range(WIN):
                b = HALO + r0 - DIL * w
                P.append(tree_sum([q[j] * k_s[j, b:b + R, :] for j in range(8)]))
            z0 = merge(merge(P[0], P[1], m16, 16), merge(P[2], P[3], m16, 16), m1, 1)
            z1 = merge(merge(P[4], P[5], m16, 16), merge(P[6], P[7], m16, 16), m1, 1)
            if r0 < DIL * (WIN - 1):
                lane = lax.broadcasted_iota(jnp.int32, shp, 1)
                row = lax.broadcasted_iota(jnp.int32, shp, 0) + (r0 + step * SB)
                w0 = ((lane >> 4) & 1) + 2 * (lane & 1)
                z0 = jnp.where(row >= DIL * w0, z0, NEG / (DH ** -0.5))
                z1 = jnp.where(row >= DIL * (w0 + 4), z1, NEG / (DH ** -0.5))
            mx = jnp.maximum(z0, z1)
            mx = jnp.maximum(mx, swap(mx, m16, 16))
            mx = jnp.maximum(mx, swap(mx, m1, 1))
            e0 = jnp.exp2((z0 - mx) * CEXP)
            e1 = jnp.exp2((z1 - mx) * CEXP)
            den = e0 + e1
            den = den + swap(den, m16, 16)
            den = den + swap(den, m1, 1)
            r = 1.0 / den
            a = []
            for e in (e0 * r, e1 * r):
                u0 = jnp.where(m1, e, _roll(e, 1))
                u1 = jnp.where(m1, _roll(e, -1), e)
                for u in (u0, u1):
                    a.append(jnp.where(m16, u, _roll(u, 16)))
                    a.append(jnp.where(m16, _roll(u, -16), u))
            outs = []
            for j in range(8):
                outs.append(tree_sum([a[w] * v_s[j, HALO + r0 - DIL * w:HALO + r0 - DIL * w + R, :] for w in range(WIN)]))
            return jnp.concatenate(outs, axis=1)

        once(prep_qkv)
        qkv_proj()

        n_rg = SB // R
        o_parts = []
        acc = None
        for f in range(nF):
            lo, hi = (n_rg * f) // nF, (n_rg * (f + 1)) // nF
            for g in range(lo, hi):
                o_parts.append(attn_rows(g * R))

            @once
            def _w():
                cp_g(f).wait()
                cp_u(f).wait()
                cp_d(f).wait()

            gt = jnp.dot(xn, wg_v[:, f * FC:(f + 1) * FC], preferred_element_type=f32)
            up = jnp.dot(xn, wu_v[:, f * FC:(f + 1) * FC], preferred_element_type=f32)
            h = (gt * jax.nn.sigmoid(gt) * up).astype(bf16)
            d = jnp.dot(h, wd_v[f * FC:(f + 1) * FC, :], preferred_element_type=f32)
            acc = d if acc is None else acc + d

        k_s[:, 0:HALO, :] = k_s[:, SB:SB + HALO, :]
        v_s[:, 0:HALO, :] = v_s[:, SB:SB + HALO, :]

        once(prep_wo)
        o = jnp.concatenate(o_parts, axis=0).astype(bf16)
        wo_p = jnp.concatenate(
            [jnp.concatenate([pltpu.bitcast(wop[ct, WOP * j:WOP * j + 64, :], bf16) for ct in range(8)], axis=1)
             for j in range(8)], axis=0)
        s = jnp.dot(o, wo_p, preferred_element_type=f32)
        out_ref[...] = (x_ref[...].astype(f32) + s * (acc * jax.nn.sigmoid(acc))).astype(out_ref.dtype)

    def run(A_x, A_wqkv, A_wo, B_w_gate, B_w_up, B_w_down):
        x2 = A_x.reshape(S, D)
        any_spec = pl.BlockSpec(memory_space=pl.ANY)
        out = pl.pallas_call(
            kernel,
            grid=(nS,),
            in_specs=[pl.BlockSpec((SB, D), lambda i: (i, 0))] + [any_spec] * 5,
            out_specs=pl.BlockSpec((SB, D), lambda i: (i, 0)),
            out_shape=jax.ShapeDtypeStruct((S, D), bf16),
            scratch_shapes=[
                pltpu.VMEM((D, 3 * D), bf16), pltpu.VMEM((D, D), bf16),
                pltpu.VMEM((D, F), bf16), pltpu.VMEM((D, F), bf16), pltpu.VMEM((F, D), bf16),
                pltpu.VMEM((D // 2, 3 * D), u32), pltpu.VMEM((8, 8 * WOP, 128), u32),
                pltpu.VMEM((8, SB, 128), f32), pltpu.VMEM((8, HALO + SB, 128), f32), pltpu.VMEM((8, HALO + SB, 128), f32),
                pltpu.SemaphoreType.DMA((2 + 3 * nF,)),
            ],
            compiler_params=pltpu.CompilerParams(dimension_semantics=("arbitrary",), vmem_limit_bytes=110 << 20),
            name="fused",
        )(x2, A_wqkv, A_wo, B_w_gate, B_w_up, B_w_down)
        return out.reshape(1, S, D)

    return run


@jax.jit
def pallas_recurrent_scan__sliding_local_dilated__swiglu_ffn__prompt_kernel(
    A_x: jax.Array,
    A_wqkv: jax.Array,
    A_wo: jax.Array,
    B_x: jax.Array,
    B_w_gate: jax.Array,
    B_w_up: jax.Array,
    B_w_down: jax.Array,
):
    del B_x
    return make_kernel()(A_x, A_wqkv, A_wo, B_w_gate, B_w_up, B_w_down)
```

```python
import functools
import math

import jax
import jax.numpy as jnp
import numpy as np
from jax import lax
from jax.experimental import pallas as pl
from jax.experimental.pallas import tpu as pltpu

S, D, F = 2048, 1024, 3584
H, DH, WIN, DIL = 32, 32, 8, 2
EPS = 1e-5
HALO = 16
bf16, f32, u32 = jnp.bfloat16, jnp.float32, jnp.uint32
NEG = -1e9
WOP = 65
BFLY = ((1, 2), (2, 4), (4, 8))


def _roll(x, s):
    return pltpu.roll(x, s % 128, 1)


def _lanebit_clear(shape, bit):
    return (lax.broadcasted_iota(jnp.int32, shape, 1) & bit) == 0


def _butterfly(t):
    for tb, lb in BFLY:
        msk = _lanebit_clear(t[0].shape, lb)
        n = [None] * 8
        for a in range(8):
            if a & tb:
                continue
            b = a | tb
            n[a] = jnp.where(msk, t[a], _roll(t[b], lb))
            n[b] = jnp.where(msk, _roll(t[a], -lb), t[b])
        t = n
    return t


class _Null:
    def __enter__(self):
        return self

    def __exit__(self, *a):
        return False


def make_kernel(SB=256, FC=512, R=8, nsteps=None, swp=False, scopes=False, qc=512, wo_pos=7, a0=0,
                attn_first=True, slab=64, prep_rows=8, ln_skew=True, skip_a=False, skip_b=False):
    nS = nsteps or S // SB
    nF = F // FC
    KP = D // 2
    nslab = KP // slab

    def kernel(x_hbm, wqkv_hbm, wo_hbm, wg_hbm, wu_hbm, wd_hbm, out_hbm,
               x_v, xn_v, out_v, wp, wo_v, wg_v, wu_v, wd_v, wop, q_s, k_s, v_s, sems):
        SEM_X0, SEM_XR, SEM_OUT, SEM_O, SEM_G, SEM_U, SEM_D, SEM_Q = range(8)

        def rd(ref, r0, r1, c0, c1):
            return pltpu.bitcast(ref[r0 // 2:r1 // 2, c0:c1], bf16)

        nx0 = min(2, nS) * SB

        def cp_x0():
            return pltpu.make_async_copy(x_hbm.at[pl.ds(0, nx0)], x_v.at[pl.ds(0, nx0)], sems.at[SEM_X0])

        def cp_xr():
            return pltpu.make_async_copy(x_hbm.at[pl.ds(nx0, nS * SB - nx0)], x_v.at[pl.ds(nx0, nS * SB - nx0)], sems.at[SEM_XR])

        def cp_q(i):
            m, sl = i // nslab, i % nslab
            return pltpu.make_async_copy(
                wqkv_hbm.bitcast(u32).at[pl.ds(sl * slab, slab), pl.ds(m * D, D)],
                wp.at[pl.ds(sl * slab, slab), pl.ds(m * D, D)], sems.at[SEM_Q + i])

        def cp_o():
            return pltpu.make_async_copy(wo_hbm.bitcast(u32), wo_v, sems.at[SEM_O])

        def cp_g():
            return pltpu.make_async_copy(wg_hbm.bitcast(u32), wg_v, sems.at[SEM_G])

        def cp_u():
            return pltpu.make_async_copy(wu_hbm.bitcast(u32), wu_v, sems.at[SEM_U])

        def cp_d():
            return pltpu.make_async_copy(wd_hbm.bitcast(u32), wd_v, sems.at[SEM_D])

        def cp_out(r0):
            return pltpu.make_async_copy(out_v.at[pl.ds(r0, SB)], out_hbm.at[pl.ds(r0, SB)], sems.at[SEM_OUT])

        def prep_wo():
            for ct in range(8):
                for T in range(8):
                    blk = wo_v[64 * T:64 * (T + 1), 128 * ct:128 * (ct + 1)]
                    for c in range(8):
                        wop[ct, pl.ds(8 * c + T, 8, stride=WOP), :] = blk[8 * c:8 * c + 8, :]

        def prep_slab(i):
            m, sl = i // nslab, i % nslab
            for p0 in range(sl * slab, (sl + 1) * slab, prep_rows):
                t = [wp[p0:p0 + prep_rows, m * D + 128 * j:m * D + 128 * (j + 1)] for j in range(8)]
                t = _butterfly(t)
                for j in range(8):
                    wp[p0:p0 + prep_rows, m * D + 128 * j:m * D + 128 * (j + 1)] = t[j]

        shp = (R, 128)
        CEXP = (DH ** -0.5) * math.log2(math.e)

        def scope(name):
            return jax.named_scope(name) if scopes else _Null()

        def layernorm(r_off):
            x = x_v[pl.ds(r_off, SB), :].astype(f32)
            mean = jnp.mean(x, axis=-1, keepdims=True)
            xc = x - mean
            var = jnp.mean(xc * xc, axis=-1, keepdims=True)
            xn_v[pl.ds(r_off, SB), :] = (xc * lax.rsqrt(var + EPS)).astype(bf16)

        def body_a(b):
            r_off = pl.multiple_of(b * SB, SB)
            if ln_skew:
                xn = xn_v[pl.ds(r_off, SB), :]
                nxt = pl.multiple_of(jnp.minimum(b + 1, nS - 1) * SB, SB)
                if nS > 1:
                    layernorm(nxt)
            else:
                layernorm(r_off)
                xn = xn_v[pl.ds(r_off, SB), :]
            for m, dst, halo in ((0, q_s, 0), (1, k_s, HALO), (2, v_s, HALO)):
                for i in range(D // qc):
                    ci = m * (D // qc) + i
                    y = jnp.dot(xn, rd(wp, 0, D, ci * qc, (ci + 1) * qc), preferred_element_type=f32)
                    for jj in range(qc // 128):
                        dst[i * (qc // 128) + jj, pl.ds(r_off + halo, SB), :] = y[:, 128 * jj:128 * (jj + 1)]

        def body_b(b):
            r_off = pl.multiple_of(b * SB, SB)
            m16 = _lanebit_clear(shp, 16)
            m1 = _lanebit_clear(shp, 1)
            xn = xn_v[pl.ds(r_off, SB), :]

            def swap(z, msk, s):
                return jnp.where(msk, _roll(z, -s), _roll(z, s))

            def merge(a, b_, msk, s):
                return jnp.where(msk, a + _roll(a, -s), b_ + _roll(b_, s))

            def tree_sum(ts):
                while len(ts) > 1:
                    ts = [ts[i] + ts[i + 1] for i in range(0, len(ts), 2)]
                return ts[0]

            def attn_rows(r0):
                q = [q_s[j, pl.ds(r_off + r0, R), :] for j in range(8)]
                P = []
                for w in range(WIN):
                    base = r_off + (HALO + r0 - DIL * w)
                    P.append(tree_sum([q[j] * k_s[j, pl.ds(base, R), :] for j in range(8)]))
                z0 = merge(merge(P[0], P[1], m16, 16), merge(P[2], P[3], m16, 16), m1, 1)
                z1 = merge(merge(P[4], P[5], m16, 16), merge(P[6], P[7], m16, 16), m1, 1)
                if r0 < DIL * (WIN - 1):
                    lane = lax.broadcasted_iota(jnp.int32, shp, 1)
                    row = lax.broadcasted_iota(jnp.int32, shp, 0) + (r0 + r_off)
                    w0 = ((lane >> 4) & 1) + 2 * (lane & 1)
                    z0 = jnp.where(row >= DIL * w0, z0, NEG / (DH ** -0.5))
                    z1 = jnp.where(row >= DIL * (w0 + 4), z1, NEG / (DH ** -0.5))
                mx = jnp.maximum(z0, z1)
                mx = jnp.maximum(mx, swap(mx, m16, 16))
                mx = jnp.maximum(mx, swap(mx, m1, 1))
                e0 = jnp.exp2((z0 - mx) * CEXP)
                e1 = jnp.exp2((z1 - mx) * CEXP)
                den = e0 + e1
                den = den + swap(den, m16, 16)
                den = den + swap(den, m1, 1)
                r = 1.0 / den
                a = []
                for e in (e0 * r, e1 * r):
                    u0 = jnp.where(m1, e, _roll(e, 1))
                    u1 = jnp.where(m1, _roll(e, -1), e)
                    for u in (u0, u1):
                        a.append(jnp.where(m16, u, _roll(u, 16)))
                        a.append(jnp.where(m16, _roll(u, -16), u))
                outs = []
                for j in range(8):
                    outs.append(tree_sum([a[w] * v_s[j, pl.ds(r_off + (HALO + r0 - DIL * w), R), :] for w in range(WIN)]))
                return jnp.concatenate(outs, axis=1)

            def gate_up(f):
                gt = jnp.dot(xn, rd(wg_v, 0, D, f * FC, (f + 1) * FC), preferred_element_type=f32)
                up = jnp.dot(xn, rd(wu_v, 0, D, f * FC, (f + 1) * FC), preferred_element_type=f32)
                return (gt * jax.nn.sigmoid(gt) * up).astype(bf16)

            def down(f, h):
                return jnp.dot(h, rd(wd_v, f * FC, (f + 1) * FC, 0, D), preferred_element_type=f32)

            def wo_dot(o_parts):
                o = jnp.concatenate(o_parts, axis=0).astype(bf16)
                wo_p = jnp.concatenate(
                    [jnp.concatenate([pltpu.bitcast(wop[ct, WOP * j:WOP * j + 64, :], bf16) for ct in range(8)], axis=1)
                     for j in range(8)], axis=0)
                return jnp.dot(o, wo_p, preferred_element_type=f32)

            n_rg = SB // R
            o_parts = []
            acc = None
            s = None
            nA = min(nF, wo_pos)
            pend = None
            for f in range(nF):
                if f == wo_pos:
                    with scope("wo"):
                        s = wo_dot(o_parts)
                with scope(f"f{f}"):
                    def do_attn():
                        if a0 <= f < nA:
                            lo, hi = (n_rg * (f - a0)) // (nA - a0), (n_rg * (f + 1 - a0)) // (nA - a0)
                            for g in range(lo, hi):
                                o_parts.append(attn_rows(g * R))

                    if attn_first:
                        do_attn()
                    h = gate_up(f)
                    if not attn_first:
                        do_attn()
                    if swp:
                        if pend is not None:
                            d = down(*pend)
                            acc = d if acc is None else acc + d
                        pend = (f, h)
                    else:
                        d = down(f, h)
                        acc = d if acc is None else acc + d
            if swp:
                d = down(*pend)
                acc = acc + d
            if s is None:
                with scope("wo"):
                    s = wo_dot(o_parts)
            with scope("comb"):
                xr = x_v[pl.ds(r_off, SB), :].astype(f32)
                out_v[pl.ds(r_off, SB), :] = (xr + s * (acc * jax.nn.sigmoid(acc))).astype(out_v.dtype)
            cp_out(r_off).start()

        cp_x0().start()
        for i in range(3 * nslab):
            cp_q(i).start()
        if nS * SB > nx0:
            cp_xr().start()
        cp_g().start()
        cp_u().start()
        cp_d().start()
        cp_o().start()
        z = jnp.zeros((8, HALO, 128), f32)
        k_s[:, 0:HALO, :] = z
        v_s[:, 0:HALO, :] = z
        with scope("x0"):
            cp_x0().wait()
            if ln_skew:
                layernorm(0)
        with scope("prep"):
            for i in range(3 * nslab):
                cp_q(i).wait()
                prep_slab(i)

        def loop_a(b, c):
            if nS * SB > nx0:
                @pl.when(b == (1 if ln_skew else 2))
                def _():
                    cp_xr().wait()
            with scope("A"):
                body_a(b)
            return c

        lax.fori_loop(0, 0 if skip_a else nS, loop_a, 0)
        if skip_a and nS * SB > nx0:
            cp_xr().wait()
        with scope("wait_w"):
            cp_g().wait()
            cp_u().wait()
            cp_d().wait()
            cp_o().wait()
            prep_wo()

        def loop_b(b, c):
            with scope("B"):
                body_b(b)
            return c

        lax.fori_loop(0, 0 if skip_b else nS, loop_b, 0)
        with scope("wait_out"):
            for i in range(0 if skip_b else nS):
                cp_out(i * SB).wait()

    def run(A_x, A_wqkv, A_wo, B_w_gate, B_w_up, B_w_down):
        x2 = A_x.reshape(S, D)
        any_spec = pl.BlockSpec(memory_space=pl.ANY)
        out = pl.pallas_call(
            kernel,
            in_specs=[any_spec] * 6,
            out_specs=any_spec,
            out_shape=jax.ShapeDtypeStruct((S, D), bf16),
            scratch_shapes=[
                pltpu.VMEM((S, D), bf16), pltpu.VMEM((S, D), bf16), pltpu.VMEM((S, D), bf16),
                pltpu.VMEM((D // 2, 3 * D), u32), pltpu.VMEM((D // 2, D), u32),
                pltpu.VMEM((D // 2, F), u32), pltpu.VMEM((D // 2, F), u32), pltpu.VMEM((F // 2, D), u32),
                pltpu.VMEM((8, 8 * WOP, 128), u32),
                pltpu.VMEM((8, S, 128), f32), pltpu.VMEM((8, HALO + S, 128), f32), pltpu.VMEM((8, HALO + S, 128), f32),
                pltpu.SemaphoreType.DMA((7 + 3 * nslab,)),
            ],
            compiler_params=pltpu.CompilerParams(vmem_limit_bytes=120 << 20),
            name="fused",
        )(x2, A_wqkv, A_wo, B_w_gate, B_w_up, B_w_down)
        return out.reshape(1, S, D)

    return run


@jax.jit
def pallas_recurrent_scan__sliding_local_dilated__swiglu_ffn__prompt_kernel(
    A_x: jax.Array,
    A_wqkv: jax.Array,
    A_wo: jax.Array,
    B_x: jax.Array,
    B_w_gate: jax.Array,
    B_w_up: jax.Array,
    B_w_down: jax.Array,
):
    del B_x
    return make_kernel(prep_rows=128, slab=128)(A_x, A_wqkv, A_wo, B_w_gate, B_w_up, B_w_down)
```

```python
import functools
import math

import jax
import jax.numpy as jnp
import numpy as np
from jax import lax
from jax.experimental import pallas as pl
from jax.experimental.pallas import tpu as pltpu

S, D, F = 2048, 1024, 3584
H, DH, WIN, DIL = 32, 32, 8, 2
EPS = 1e-5
HALO = 16
bf16, f32, u32 = jnp.bfloat16, jnp.float32, jnp.uint32
NEG = -1e9
WOP = 65
BFLY = ((1, 2), (2, 4), (4, 8))


def _roll(x, s):
    return pltpu.roll(x, s % 128, 1)


def _lanebit_clear(shape, bit):
    return (lax.broadcasted_iota(jnp.int32, shape, 1) & bit) == 0


def _butterfly(t):
    for tb, lb in BFLY:
        msk = _lanebit_clear(t[0].shape, lb)
        n = [None] * 8
        for a in range(8):
            if a & tb:
                continue
            b = a | tb
            n[a] = jnp.where(msk, t[a], _roll(t[b], lb))
            n[b] = jnp.where(msk, _roll(t[a], -lb), t[b])
        t = n
    return t


class _Null:
    def __enter__(self):
        return self

    def __exit__(self, *a):
        return False


def make_kernel(SB=256, FC=512, R=8, swp=False, scopes=False, qc=512, wo_pos=7, a0=0,
                attn_first=True, slab=128, SBA=256, skip_b=False, nb_steps=None, a0_order='qlp', wo_split=None, dep=False, flags=None, ev=False):
    if ev:
        flags = dict(flags or {}, XLA_TPU_EVENLY_DISTRIBUTE_CRITICAL_NODES=True)
    nS = S // SB
    nF = F // FC
    KP = D // 2
    nslab = KP // slab
    assert 2 * nslab == nS

    def kernel(x_hbm, wqkv_hbm, wo_hbm, wg_hbm, wu_hbm, wd_hbm, out_hbm,
               x_v, xn_v, out_v, wq_v, wkv_v, wo_v, wg_v, wu_v, wd_v, wop, q_s, k_s, v_s, z_ref, sems):
        SEM_OUT, SEM_O, SEM_G, SEM_U, SEM_D = range(5)
        SEM_X = 5
        SEM_Q = 5 + nS

        def rd(ref, r0, r1, c0, c1):
            return pltpu.bitcast(ref[r0 // 2:r1 // 2, c0:c1], bf16)

        def cp_x(i):
            r0 = i * SB if isinstance(i, int) else pl.multiple_of(i * SB, SB)
            return pltpu.make_async_copy(x_hbm.at[pl.ds(r0, SB)], x_v.at[pl.ds(r0, SB)], sems.at[SEM_X + i])

        def slab_pos(i):
            if isinstance(i, int):
                return (i % nslab) * slab, (i // nslab) * D
            return pl.multiple_of((i % nslab) * slab, slab), pl.multiple_of((i // nslab) * D, D)

        def cp_q(i):
            p0, _ = slab_pos(i)
            return pltpu.make_async_copy(wqkv_hbm.bitcast(u32).at[pl.ds(p0, slab), pl.ds(0, D)],
                                         wq_v.at[pl.ds(p0, slab), :], sems.at[SEM_Q + i])

        def cp_kv(i):
            p0, c0 = slab_pos(i)
            return pltpu.make_async_copy(wqkv_hbm.bitcast(u32).at[pl.ds(p0, slab), pl.ds(D + c0, D)],
                                         wkv_v.at[pl.ds(p0, slab), pl.ds(c0, D)], sems.at[SEM_Q + nslab + i])

        def cp_o():
            return pltpu.make_async_copy(wo_hbm.bitcast(u32), wo_v, sems.at[SEM_O])

        def cp_g():
            return pltpu.make_async_copy(wg_hbm.bitcast(u32), wg_v, sems.at[SEM_G])

        def cp_u():
            return pltpu.make_async_copy(wu_hbm.bitcast(u32), wu_v, sems.at[SEM_U])

        def cp_d():
            return pltpu.make_async_copy(wd_hbm.bitcast(u32), wd_v, sems.at[SEM_D])

        def cp_out(r0):
            return pltpu.make_async_copy(out_v.at[pl.ds(r0, SB)], out_hbm.at[pl.ds(r0, SB)], sems.at[SEM_OUT])

        def prep_wo():
            for ct in range(8):
                for T in range(8):
                    blk = wo_v[64 * T:64 * (T + 1), 128 * ct:128 * (ct + 1)]
                    for c in range(8):
                        wop[ct, pl.ds(8 * c + T, 8, stride=WOP), :] = blk[8 * c:8 * c + 8, :]

        def prep_slab(ref, i):
            p0, c0 = slab_pos(i)
            t = [ref[pl.ds(p0, slab), pl.ds(c0 + 128 * j, 128)] for j in range(8)]
            t = _butterfly(t)
            for j in range(8):
                ref[pl.ds(p0, slab), pl.ds(c0 + 128 * j, 128)] = t[j]

        shp = (R, 128)
        CEXP = (DH ** -0.5) * math.log2(math.e)

        def scope(name):
            if scopes == 1 and name[0] in "fwc" and name not in ("wait_w", "wait_out"):
                return _Null()
            return jax.named_scope(name) if scopes else _Null()

        def layernorm(r_off):
            x = x_v[pl.ds(r_off, SB), :].astype(f32)
            mean = jnp.mean(x, axis=-1, keepdims=True)
            xc = x - mean
            var = jnp.mean(xc * xc, axis=-1, keepdims=True)
            xn_v[pl.ds(r_off, SB), :] = (xc * lax.rsqrt(var + EPS)).astype(bf16)

        def proj(xn, wref, m, dst, row0, nrows):
            for i in range(D // qc):
                ci = m * (D // qc) + i
                y = jnp.dot(xn, rd(wref, 0, D, ci * qc, (ci + 1) * qc), preferred_element_type=f32)
                for jj in range(qc // 128):
                    dst[i * (qc // 128) + jj, pl.ds(row0, nrows), :] = y[:, 128 * jj:128 * (jj + 1)]

        def body_a0(b):
            r_off = pl.multiple_of(b * SB, SB)
            nxt = jnp.minimum(b + 1, nS - 1)

            @pl.when(b < nS - 1)
            def _():
                cp_x(b + 1).wait()
            cp_kv(b).wait()
            xn = xn_v[pl.ds(r_off, SB), :]
            steps = {"p": lambda: prep_slab(wkv_v, b), "l": lambda: layernorm(pl.multiple_of(nxt * SB, SB)),
                     "q": lambda: proj(xn, wq_v, 0, q_s, r_off, SB)}
            for c in a0_order:
                steps[c]()

        def body_a1(b):
            r_off = pl.multiple_of(b * SBA, SBA)
            xn = xn_v[pl.ds(r_off, SBA), :]
            proj(xn, wkv_v, 0, k_s, r_off + HALO, SBA)
            proj(xn, wkv_v, 1, v_s, r_off + HALO, SBA)

        def body_b(b):
            r_off = pl.multiple_of(b * SB, SB)
            m16 = _lanebit_clear(shp, 16)
            m1 = _lanebit_clear(shp, 1)
            xn = xn_v[pl.ds(r_off, SB), :]

            def swap(z, msk, s):
                return jnp.where(msk, _roll(z, -s), _roll(z, s))

            def merge(a, b_, msk, s):
                return jnp.where(msk, a + _roll(a, -s), b_ + _roll(b_, s))

            def tree_sum(ts):
                while len(ts) > 1:
                    ts = [ts[i] + ts[i + 1] for i in range(0, len(ts), 2)]
                return ts[0]

            def attn_rows(r0):
                q = [q_s[j, pl.ds(r_off + r0, R), :] for j in range(8)]
                P = []
                for w in range(WIN):
                    base = r_off + (HALO + r0 - DIL * w)
                    P.append(tree_sum([q[j] * k_s[j, pl.ds(base, R), :] for j in range(8)]))
                z0 = merge(merge(P[0], P[1], m16, 16), merge(P[2], P[3], m16, 16), m1, 1)
                z1 = merge(merge(P[4], P[5], m16, 16), merge(P[6], P[7], m16, 16), m1, 1)
                if r0 < DIL * (WIN - 1):
                    lane = lax.broadcasted_iota(jnp.int32, shp, 1)
                    row = lax.broadcasted_iota(jnp.int32, shp, 0) + (r0 + r_off)
                    w0 = ((lane >> 4) & 1) + 2 * (lane & 1)
                    z0 = jnp.where(row >= DIL * w0, z0, NEG / (DH ** -0.5))
                    z1 = jnp.where(row >= DIL * (w0 + 4), z1, NEG / (DH ** -0.5))
                mx = jnp.maximum(z0, z1)
                mx = jnp.maximum(mx, swap(mx, m16, 16))
                mx = jnp.maximum(mx, swap(mx, m1, 1))
                e0 = jnp.exp2((z0 - mx) * CEXP)
                e1 = jnp.exp2((z1 - mx) * CEXP)
                den = e0 + e1
                den = den + swap(den, m16, 16)
                den = den + swap(den, m1, 1)
                r = 1.0 / den
                a = []
                for e in (e0 * r, e1 * r):
                    u0 = jnp.where(m1, e, _roll(e, 1))
                    u1 = jnp.where(m1, _roll(e, -1), e)
                    for u in (u0, u1):
                        a.append(jnp.where(m16, u, _roll(u, 16)))
                        a.append(jnp.where(m16, _roll(u, -16), u))
                outs = []
                for j in range(8):
                    outs.append(tree_sum([a[w] * v_s[j, pl.ds(r_off + (HALO + r0 - DIL * w), R), :] for w in range(WIN)]))
                return jnp.concatenate(outs, axis=1)

            def gate_up(f):
                gt = jnp.dot(xn, rd(wg_v, 0, D, f * FC, (f + 1) * FC), preferred_element_type=f32)
                up = jnp.dot(xn, rd(wu_v, 0, D, f * FC, (f + 1) * FC), preferred_element_type=f32)
                return (gt * jax.nn.sigmoid(gt) * up).astype(bf16)

            def down(f, h):
                return jnp.dot(h, rd(wd_v, f * FC, (f + 1) * FC, 0, D), preferred_element_type=f32)

            def wo_dot(o_parts):
                o = jnp.concatenate(o_parts, axis=0).astype(bf16)
                wo_p = jnp.concatenate(
                    [jnp.concatenate([pltpu.bitcast(wop[ct, WOP * j:WOP * j + 64, :], bf16) for ct in range(8)], axis=1)
                     for j in range(8)], axis=0)
                return jnp.dot(o, wo_p, preferred_element_type=f32)

            n_rg = SB // R
            o_parts = []
            acc = None
            s = None
            nA = min(nF, wo_pos)
            pend = None
            s_parts = []
            nsplit = len(wo_split) if wo_split else 0
            if dep:
                zmask = z_ref[...]
            last_new = []
            for f in range(nF):
                if f == wo_pos and not wo_split:
                    with scope("wo"):
                        s = wo_dot(o_parts)
                if wo_split and f in wo_split:
                    i = wo_split.index(f)
                    while len(o_parts) < (i + 1) * n_rg // nsplit:
                        o_parts.append(attn_rows(len(o_parts) * R))
                    s_parts.append(wo_dot(o_parts[i * n_rg // nsplit:(i + 1) * n_rg // nsplit]))
                with scope(f"f{f}"):
                    def do_attn():
                        new = []
                        if wo_split:
                            return new
                        if a0 <= f < nA:
                            lo, hi = (n_rg * (f - a0)) // (nA - a0), (n_rg * (f + 1 - a0)) // (nA - a0)
                            for g in range(lo, hi):
                                o_parts.append(attn_rows(g * R))
                                new.append(o_parts[-1])
                        return new

                    if attn_first:
                        new = do_attn()
                    h = gate_up(f)
                    if not attn_first:
                        new = do_attn()
                    if dep and last_new:
                        t = None
                        for piece in last_new:
                            for j in range(8):
                                pb = pltpu.bitcast(piece[:, 128 * j:128 * (j + 1)], u32)
                                t = pb if t is None else t | pb
                        hb = pltpu.bitcast(h, u32)
                        top = jnp.concatenate([hb[0:8, 0:128] | (t & zmask), hb[0:8, 128:]], axis=1)
                        h = pltpu.bitcast(jnp.concatenate([top, hb[8:, :]], axis=0), bf16)
                    last_new = new
                    if swp:
                        if pend is not None:
                            d = down(*pend)
                            acc = d if acc is None else acc + d
                        pend = (f, h)
                    else:
                        d = down(f, h)
                        acc = d if acc is None else acc + d
            if swp:
                d = down(*pend)
                acc = acc + d
            if wo_split:
                i = len(s_parts)
                if i < nsplit:
                    while len(o_parts) < n_rg:
                        o_parts.append(attn_rows(len(o_parts) * R))
                    s_parts.append(wo_dot(o_parts[i * n_rg // nsplit:]))
                s = jnp.concatenate(s_parts, axis=0)
            if s is None:
                with scope("wo"):
                    s = wo_dot(o_parts)
            with scope("comb"):
                xr = x_v[pl.ds(r_off, SB), :].astype(f32)
                out_v[pl.ds(r_off, SB), :] = (xr + s * (acc * jax.nn.sigmoid(acc))).astype(out_v.dtype)
            cp_out(r_off).start()

        cp_x(0).start()
        for i in range(nslab):
            cp_q(i).start()
        for b_ in range(nS):
            if b_ + 1 < nS:
                cp_x(b_ + 1).start()
            cp_kv(b_).start()
        cp_g().start()
        cp_u().start()
        cp_d().start()
        cp_o().start()
        z_ref[...] = jnp.zeros((8, 128), u32)
        z = jnp.zeros((8, HALO, 128), f32)
        k_s[:, 0:HALO, :] = z
        v_s[:, 0:HALO, :] = z
        with scope("x0"):
            cp_x(0).wait()
            layernorm(0)

        def loop_prep(i, c):
            cp_q(i).wait()
            prep_slab(wq_v, i)
            return c

        with scope("prep"):
            lax.fori_loop(0, nslab, loop_prep, 0)

        def loop_a0(b, c):
            with scope("A0"):
                body_a0(b)
            return c

        lax.fori_loop(0, nS, loop_a0, 0)

        def loop_a1(b, c):
            with scope("A1"):
                body_a1(b)
            return c

        lax.fori_loop(0, S // SBA, loop_a1, 0)
        with scope("wait_w"):
            cp_g().wait()
            cp_u().wait()
            cp_d().wait()
            cp_o().wait()
            prep_wo()

        def loop_b(b, c):
            with scope("B"):
                body_b(b)
            return c

        nb = 0 if skip_b else (nb_steps or nS)
        lax.fori_loop(0, nb, loop_b, 0)
        with scope("wait_out"):
            for i in range(nb):
                cp_out(i * SB).wait()

    def run(A_x, A_wqkv, A_wo, B_w_gate, B_w_up, B_w_down):
        x2 = A_x.reshape(S, D)
        any_spec = pl.BlockSpec(memory_space=pl.ANY)
        out = pl.pallas_call(
            kernel,
            in_specs=[any_spec] * 6,
            out_specs=any_spec,
            out_shape=jax.ShapeDtypeStruct((S, D), bf16),
            scratch_shapes=[
                pltpu.VMEM((S, D), bf16), pltpu.VMEM((S, D), bf16), pltpu.VMEM((S, D), bf16),
                pltpu.VMEM((D // 2, D), u32), pltpu.VMEM((D // 2, 2 * D), u32), pltpu.VMEM((D // 2, D), u32),
                pltpu.VMEM((D // 2, F), u32), pltpu.VMEM((D // 2, F), u32), pltpu.VMEM((F // 2, D), u32),
                pltpu.VMEM((8, 8 * WOP, 128), u32),
                pltpu.VMEM((8, S, 128), f32), pltpu.VMEM((8, HALO + S, 128), f32), pltpu.VMEM((8, HALO + S, 128), f32),
                pltpu.VMEM((8, 128), u32),
                pltpu.SemaphoreType.DMA((5 + nS + 3 * nslab,)),
            ],
            compiler_params=pltpu.CompilerParams(vmem_limit_bytes=120 << 20, flags=flags),
            name="fused",
        )(x2, A_wqkv, A_wo, B_w_gate, B_w_up, B_w_down)
        return out.reshape(1, S, D)

    return run


@jax.jit
def pallas_recurrent_scan__sliding_local_dilated__swiglu_ffn__prompt_kernel(
    A_x: jax.Array,
    A_wqkv: jax.Array,
    A_wo: jax.Array,
    B_x: jax.Array,
    B_w_gate: jax.Array,
    B_w_up: jax.Array,
    B_w_down: jax.Array,
):
    del B_x
    return make_kernel(ev=True, SBA=512)(A_x, A_wqkv, A_wo, B_w_gate, B_w_up, B_w_down)
```

```python
import functools
import math

import jax
import jax.numpy as jnp
import numpy as np
from jax import lax
from jax.experimental import pallas as pl
from jax.experimental.pallas import tpu as pltpu

S, D, F = 2048, 1024, 3584
H, DH, WIN, DIL = 32, 32, 8, 2
EPS = 1e-5
HALO = 16
NEG = -1e9
bf16, f32, u32 = jnp.bfloat16, jnp.float32, jnp.uint32
WOP = 65
BFLY = ((1, 2), (2, 4), (4, 8))
DP, DHALF = D // 2, D // 2
KP = D // 4


def _roll(x, s):
    return pltpu.roll(x, s % 128, 1)


def _lanebit_clear(shape, bit):
    return (lax.broadcasted_iota(jnp.int32, shape, 1) & bit) == 0


def _butterfly(t):
    for tb, lb in BFLY:
        msk = _lanebit_clear(t[0].shape, lb)
        n = [None] * 8
        for a in range(8):
            if a & tb:
                continue
            b = a | tb
            n[a] = jnp.where(msk, t[a], _roll(t[b], lb))
            n[b] = jnp.where(msk, _roll(t[a], -lb), t[b])
        t = n
    return t


def _dot(a, b):
    return jnp.dot(a, b, preferred_element_type=f32)


def _a_combos(a):
    m, k = a.shape[0] // 2, a.shape[1] // 2
    a11, a12, a21, a22 = a[:m, :k], a[:m, k:], a[m:, :k], a[m:, k:]
    return [t.astype(bf16) for t in (a11 + a22, a21 + a22, a11, a22, a11 + a12, a21 - a11, a12 - a22)]


def _c_combos(m):
    return (m[0] + m[3] - m[4] + m[6], m[2] + m[4], m[1] + m[3], m[0] - m[1] + m[2] + m[5])


def _c_full(m):
    c11, c12, c21, c22 = _c_combos(m)
    return jnp.concatenate([jnp.concatenate([c11, c12], axis=1), jnp.concatenate([c21, c22], axis=1)], axis=0)


EMULATE_PACK = False


def _unpack(t, i):
    if EMULATE_PACK:
        return lax.bitcast_convert_type((t << 16) if i == 0 else (t & jnp.uint32(0xFFFF0000)), f32)
    return pltpu.unpack_elementwise(t, index=i, packed_dtype=bf16, unpacked_dtype=f32)


def _pack(lo, hi):
    if EMULATE_PACK:
        b = lambda v: lax.bitcast_convert_type(v.astype(bf16).astype(f32), u32)
        return (b(lo) >> 16) | b(hi)
    return pltpu.bitcast(pltpu.pack_elementwise([lo, hi], packed_dtype=bf16), u32)


def _b_combos(b11, b12, b21, b22):
    def half(i):
        return [_unpack(t, i) for t in (b11, b12, b21, b22)]

    def five(x11, x12, x21, x22):
        return (x11 + x22, x12 - x22, x21 - x11, x11 + x12, x21 + x22)

    return [_pack(lo, hi) for lo, hi in zip(five(*half(0)), five(*half(1)))]


def _rhs7(b11, b22, cmb):
    r = [cmb(0), b11, cmb(1), cmb(2), b22, cmb(3), cmb(4)]
    return [pltpu.bitcast(t, bf16) for t in r]


class _Null:
    def __enter__(self):
        return self

    def __exit__(self, *a):
        return False


def make_kernel(SB=256, FC=512, R=8, SBA=512, swp=False, scopes=False, ev=False, flags=None, dep=True, cslab=1,
                a0_order="qlp", nb_steps=None, st_o=True, wo_pos=7, interpret=False, a1_mode='inter'):
    nS = S // SB
    nF = F // FC
    FH = FC // 2
    HB = SB // 2
    XP = HB // 2
    NQ = S // SBA
    GR = KP // NQ
    DC = DHALF // NQ
    slab = KP // 4
    nslab = 4
    assert nS == 2 * nslab and NQ == 4 and DC % 128 == 0 and GR % 8 == 0 and FH % 128 == 0 and (FH // 2) % 8 == 0
    if ev:
        flags = dict(flags or {}, XLA_TPU_EVENLY_DISTRIBUTE_CRITICAL_NODES=True)

    def kernel(x_hbm, wqkv_hbm, wo_hbm, wg_hbm, wu_hbm, wd_hbm, out_hbm,
               x_v, xl_v, out_v, wq_v, qc_v, wkv_v, kvc_v, wo_v, wop, woc,
               wg_v, wu_v, wd_v, gc, uc, dc, q_s, k_s, v_s, z_ref, sems):
        SEM_OUT, SEM_O = 0, 1
        SEM_X = 2
        SEM_Q = SEM_X + nS
        SEM_KV = SEM_Q + nslab
        SEM_F = SEM_KV + nS

        def scope(name):
            return jax.named_scope(name) if scopes else _Null()

        def w32(ref):
            return ref if EMULATE_PACK else ref.bitcast(u32)

        def mult(v, m):
            return v if isinstance(v, int) else pl.multiple_of(v, m)

        def cp_x(i):
            r0 = mult(i * SB, SB)
            return pltpu.make_async_copy(x_hbm.at[pl.ds(r0, SB)], x_v.at[pl.ds(r0, SB)], sems.at[SEM_X + i])

        def cp_pair(dst, dst_c0, m, i, sem):
            cps = []
            for kh in range(2):
                p0 = mult(kh * KP + i * slab, slab)
                cps.append(pltpu.make_async_copy(
                    w32(wqkv_hbm).at[pl.ds(p0, slab), pl.ds(mult(m * D, D), D)],
                    dst.at[pl.ds(p0, slab), pl.ds(dst_c0, D)], sems.at[sem]))
            return cps

        def cp_q(i):
            return cp_pair(wq_v, 0, 0, i, SEM_Q + i)

        def cp_kv(b):
            m, i = b // nslab, b % nslab
            return cp_pair(wkv_v, mult(m * D, D), 1 + m, i, SEM_KV + b)

        def cp_o():
            return pltpu.make_async_copy(w32(wo_hbm), wo_v, sems.at[SEM_O])

        def cp_ffn(q):
            cps = []
            for src, dst in ((wg_hbm, wg_v), (wu_hbm, wu_v)):
                for kh in range(2):
                    r0 = mult(kh * KP + q * GR, 8)
                    cps.append(pltpu.make_async_copy(w32(src).at[pl.ds(r0, GR), :], dst.at[pl.ds(r0, GR), :], sems.at[SEM_F + q]))
            for nh in range(2):
                c0 = mult(nh * DHALF + q * DC, 128)
                cps.append(pltpu.make_async_copy(w32(wd_hbm).at[:, pl.ds(c0, DC)], wd_v.at[:, pl.ds(c0, DC)], sems.at[SEM_F + q]))
            return cps

        def cp_out(r0):
            return pltpu.make_async_copy(out_v.at[pl.ds(r0, SB)], out_hbm.at[pl.ds(r0, SB)], sems.at[SEM_OUT])

        def prep_pair(raw, c0, cmb, mi, i):
            p1 = mult(i * slab, slab)
            p2 = mult(KP + i * slab, slab)
            t1 = _butterfly([raw[pl.ds(p1, slab), pl.ds(c0 + 128 * j, 128)] for j in range(8)])
            t2 = _butterfly([raw[pl.ds(p2, slab), pl.ds(c0 + 128 * j, 128)] for j in range(8)])
            for j in range(4):
                raw[pl.ds(p1, slab), pl.ds(c0 + 128 * j, 128)] = t1[j]
                raw[pl.ds(p2, slab), pl.ds(c0 + 128 * (4 + j), 128)] = t2[4 + j]
                o = _b_combos(t1[j], t1[4 + j], t2[j], t2[4 + j])
                for k in range(5):
                    cmb[mi, k, pl.ds(p1, slab), 128 * j:128 * (j + 1)] = o[k]

        def qkv_rhs(raw, c0, cmb, mi):
            return _rhs7(raw[0:KP, c0:c0 + DHALF], raw[KP:2 * KP, c0 + DHALF:c0 + D], lambda k: cmb[mi, k])

        def tied(v, tie):
            if tie is None:
                return v
            if v.shape[0] == 8:
                return v | tie
            return jnp.concatenate([v[0:8] | tie, v[8:]], axis=0)

        def ffn_pieces(q):
            r0 = pl.multiple_of(q * GR, 8)
            c0 = pl.multiple_of(q * DC, 128)
            CR = 8 * cslab
            out = []

            def gu_piece(raw, dst, f, ct, rr, tie=None):
                cl, cr = f * FC + ct * 128, f * FC + FH + ct * 128
                o = _b_combos(tied(raw[pl.ds(r0 + rr, CR), cl:cl + 128], tie), raw[pl.ds(r0 + rr, CR), cr:cr + 128],
                              raw[pl.ds(KP + r0 + rr, CR), cl:cl + 128], raw[pl.ds(KP + r0 + rr, CR), cr:cr + 128])
                for k in range(5):
                    dst[k, pl.ds(r0 + rr, CR), f * FH + ct * 128:f * FH + (ct + 1) * 128] = o[k]

            def d_piece(f, rr, cc, tie=None):
                k0, kq = f * FH + rr, FH // 2
                o = _b_combos(tied(wd_v[k0:k0 + CR, pl.ds(c0 + cc, 128)], tie), wd_v[k0:k0 + CR, pl.ds(DHALF + c0 + cc, 128)],
                              wd_v[k0 + kq:k0 + kq + CR, pl.ds(c0 + cc, 128)], wd_v[k0 + kq:k0 + kq + CR, pl.ds(DHALF + c0 + cc, 128)])
                for k in range(5):
                    dc[k, f * kq + rr:f * kq + rr + CR, pl.ds(c0 + cc, 128)] = o[k]

            for raw, dst in ((wg_v, gc), (wu_v, uc)):
                for f in range(nF):
                    for ct in range(FH // 128):
                        for rr in range(0, GR, CR):
                            out.append(functools.partial(gu_piece, raw, dst, f, ct, rr))
            for f in range(nF):
                for cc in range(0, DC, 128):
                    for rr in range(0, FH // 2, CR):
                        out.append(functools.partial(d_piece, f, rr, cc))
            return out

        def wo_pieces(q):
            out = []

            def plane(ct, tie=None):
                c0 = pl.multiple_of(ct * 128, 128)
                for T in range(8):
                    blk = tied(wo_v[64 * T:64 * (T + 1), pl.ds(c0, 128)], tie)
                    for c in range(8):
                        wop[ct, pl.ds(8 * c + T, 8, stride=WOP), :] = blk[8 * c:8 * c + 8, :]

            def combo(jj, tie=None):
                c0 = pl.multiple_of(q * 128, 128)
                o = _b_combos(wop[q, WOP * jj:WOP * jj + 64, :], wop[4 + q, WOP * jj:WOP * jj + 64, :],
                              wop[q, WOP * (4 + jj):WOP * (4 + jj) + 64, :], wop[4 + q, WOP * (4 + jj):WOP * (4 + jj) + 64, :])
                for k in range(5):
                    woc[k, 64 * jj:64 * (jj + 1), pl.ds(c0, 128)] = o[k]

            out.append(functools.partial(plane, q))
            out.append(functools.partial(plane, 4 + q))
            if st_o:
                for jj in range(4):
                    out.append(functools.partial(combo, jj))
            return out

        def wo_tile(j0, j1, c0, c1):
            return jnp.concatenate(
                [jnp.concatenate([wop[ct, WOP * j:WOP * j + 64, :] for ct in range(c0, c1)], axis=1) for j in range(j0, j1)], axis=0)

        def layernorm(b):
            x = x_v[pl.ds(mult(b * SB, SB), SB), :].astype(f32)
            mean = jnp.mean(x, axis=-1, keepdims=True)
            xc = x - mean
            var = jnp.mean(xc * xc, axis=-1, keepdims=True)
            xn = xc * lax.rsqrt(var + EPS)
            p0 = mult(b * XP, XP)
            for k, l in enumerate(_a_combos(xn)):
                xl_v[k, pl.ds(p0, XP), :] = pltpu.bitcast(l, u32)

        def xl_lhs(p0, n):
            return [pltpu.bitcast(xl_v[k, pl.ds(p0, n), :], bf16) for k in range(7)]

        def store_planes(dst, row0, nblk, m):
            c11, c12, c21, c22 = _c_combos(m)
            for blk in range(nblk):
                for half, (cl, cr) in enumerate(((c11, c12), (c21, c22))):
                    r = row0 + blk * SB + half * HB
                    for j in range(4):
                        dst[j, pl.ds(r, HB), :] = cl[blk * HB:(blk + 1) * HB, 128 * j:128 * (j + 1)]
                        dst[4 + j, pl.ds(r, HB), :] = cr[blk * HB:(blk + 1) * HB, 128 * j:128 * (j + 1)]

        def body_a0(b):
            @pl.when(b < nS - 1)
            def _():
                cp_x(b + 1).wait()
            for cp in cp_kv(b):
                cp.wait()
            lhs = xl_lhs(pl.multiple_of(b * XP, XP), XP)
            nxt = jnp.minimum(b + 1, nS - 1)

            def q_proj():
                m = [_dot(l, w) for l, w in zip(lhs, qkv_rhs(wq_v, 0, qc_v, 0))]
                store_planes(q_s, pl.multiple_of(b * SB, SB), 1, m)

            steps = {"q": q_proj, "l": lambda: layernorm(nxt),
                     "p": lambda: prep_pair(wkv_v, pl.multiple_of((b // nslab) * D, D), kvc_v, b // nslab, b % nslab)}
            for c in a0_order:
                steps[c]()

        def body_a1(b):
            @pl.when(b == 0)
            def _():
                cp_o().wait()
            for cp in cp_ffn(b):
                cp.wait()
            nblk = SBA // SB
            lhs = xl_lhs(pl.multiple_of(b * nblk * XP, XP), nblk * XP)
            pieces = wo_pieces(b) + ffn_pieces(b)
            row0 = pl.multiple_of(b * SBA, SBA) + HALO
            prev = None

            def tie_lhs(l, tv):
                lb = pltpu.bitcast(l, u32)
                top = jnp.concatenate([lb[0:8, 0:128] | tv, lb[0:8, 128:]], axis=1)
                return pltpu.bitcast(jnp.concatenate([top, lb[8:, :]], axis=0), bf16)

            d0 = {"chain": 0, "chain2": 1, "inter": 0, "after": 0, "tie": 0, "v": 7, "end": 14, "mid": 7}[a1_mode]
            nd = 14 - d0
            grp = [[] for _ in range(15)]
            if a1_mode in ("end", "mid"):
                grp[d0] = pieces
            else:
                for i in range(nd):
                    grp[d0 + i] = pieces[(len(pieces) * i) // nd:(len(pieces) * (i + 1)) // nd]
            for mi, dst in enumerate((k_s, v_s)):
                m = []
                for k, (l, w) in enumerate(zip(lhs, qkv_rhs(wkv_v, mi * D, kvc_v, mi))):
                    if a1_mode not in ("after", "tie", "chain", "chain2"):
                        for piece in grp[7 * mi + k]:
                            piece()
                    if a1_mode in ("chain", "chain2"):
                        if prev is not None:
                            tv = pltpu.bitcast(prev[0:8, 0:128], u32) & z_ref[...]
                            l = tie_lhs(l, tv)
                        else:
                            tv = None
                        for piece in grp[7 * mi + k]:
                            piece(tie=tv)
                    m.append(_dot(l, w))
                    prev = m[-1]
                    if a1_mode == "tie":
                        tv = pltpu.bitcast(m[-1][0:8, 0:128], u32) & z_ref[...]
                        for piece in grp[7 * mi + k]:
                            piece(tie=tv)
                    if a1_mode == "after":
                        for piece in grp[7 * mi + k]:
                            piece()
                store_planes(dst, row0, nblk, m)
            for piece in grp[14]:
                piece()

        shp = (R, 128)
        CEXP = (DH ** -0.5) * math.log2(math.e)

        def body_b(b):
            r_off = pl.multiple_of(b * SB, SB)
            m16 = _lanebit_clear(shp, 16)
            m1 = _lanebit_clear(shp, 1)
            xl = xl_lhs(pl.multiple_of(b * XP, XP), XP)

            def swap(z, msk, s):
                return jnp.where(msk, _roll(z, -s), _roll(z, s))

            def merge(a, b_, msk, s):
                return jnp.where(msk, a + _roll(a, -s), b_ + _roll(b_, s))

            def tree_sum(ts):
                while len(ts) > 1:
                    ts = [ts[i] + ts[i + 1] for i in range(0, len(ts), 2)]
                return ts[0]

            def attn_rows(r0):
                q = [q_s[j, pl.ds(r_off + r0, R), :] for j in range(8)]
                P = []
                for w in range(WIN):
                    base = r_off + (HALO + r0 - DIL * w)
                    P.append(tree_sum([q[j] * k_s[j, pl.ds(base, R), :] for j in range(8)]))
                z0 = merge(merge(P[0], P[1], m16, 16), merge(P[2], P[3], m16, 16), m1, 1)
                z1 = merge(merge(P[4], P[5], m16, 16), merge(P[6], P[7], m16, 16), m1, 1)
                if r0 < DIL * (WIN - 1):
                    lane = lax.broadcasted_iota(jnp.int32, shp, 1)
                    row = lax.broadcasted_iota(jnp.int32, shp, 0) + (r0 + r_off)
                    w0 = ((lane >> 4) & 1) + 2 * (lane & 1)
                    z0 = jnp.where(row >= DIL * w0, z0, NEG / (DH ** -0.5))
                    z1 = jnp.where(row >= DIL * (w0 + 4), z1, NEG / (DH ** -0.5))
                mx = jnp.maximum(z0, z1)
                mx = jnp.maximum(mx, swap(mx, m16, 16))
                mx = jnp.maximum(mx, swap(mx, m1, 1))
                e0 = jnp.exp2((z0 - mx) * CEXP)
                e1 = jnp.exp2((z1 - mx) * CEXP)
                den = e0 + e1
                den = den + swap(den, m16, 16)
                den = den + swap(den, m1, 1)
                r = 1.0 / den
                a = []
                for e in (e0 * r, e1 * r):
                    u0 = jnp.where(m1, e, _roll(e, 1))
                    u1 = jnp.where(m1, _roll(e, -1), e)
                    for u in (u0, u1):
                        a.append(jnp.where(m16, u, _roll(u, 16)))
                        a.append(jnp.where(m16, _roll(u, -16), u))
                outs = []
                for j in range(8):
                    outs.append(tree_sum([a[w] * v_s[j, pl.ds(r_off + (HALO + r0 - DIL * w), R), :] for w in range(WIN)]))
                return jnp.concatenate(outs, axis=1)

            def gu_rhs(raw, cmb, f):
                return _rhs7(raw[0:KP, f * FC:f * FC + FH], raw[KP:2 * KP, f * FC + FH:(f + 1) * FC],
                             lambda k: cmb[k, :, f * FH:(f + 1) * FH])

            def d_rhs(f):
                k0, kq = f * FH, FH // 2
                return _rhs7(wd_v[k0:k0 + kq, 0:DHALF], wd_v[k0 + kq:k0 + 2 * kq, DHALF:D], lambda k: dc[k, f * kq:(f + 1) * kq, :])

            def gate_up(f):
                gt = _c_full([_dot(l, w) for l, w in zip(xl, gu_rhs(wg_v, gc, f))])
                up = _c_full([_dot(l, w) for l, w in zip(xl, gu_rhs(wu_v, uc, f))])
                return _a_combos(gt * jax.nn.sigmoid(gt) * up)

            def down(f, hl):
                return [_dot(l, w) for l, w in zip(hl, d_rhs(f))]

            def wo_dot(o_parts):
                o = jnp.concatenate(o_parts, axis=0)
                if st_o:
                    rhs = _rhs7(wo_tile(0, 4, 0, 4), wo_tile(4, 8, 4, 8), lambda k: woc[k])
                    return _c_full([_dot(l, w) for l, w in zip(_a_combos(o), rhs)])
                return _dot(o.astype(bf16), pltpu.bitcast(wo_tile(0, 8, 0, 8), bf16))

            def tie(lhs, pieces):
                t = None
                for piece in pieces:
                    for j in range(8):
                        pb = pltpu.bitcast(piece[:, 128 * j:128 * (j + 1)], u32)
                        t = pb if t is None else t | pb
                hb = pltpu.bitcast(lhs, u32)
                top = jnp.concatenate([hb[0:8, 0:128] | (t & z_ref[...]), hb[0:8, 128:]], axis=1)
                return pltpu.bitcast(jnp.concatenate([top, hb[8:, :]], axis=0), bf16)

            n_rg = SB // R
            last_new = []
            o_parts, acc, s, pend = [], None, None, None
            nA = min(nF, wo_pos)
            for f in range(nF):
                if f == wo_pos:
                    s = wo_dot(o_parts)
                new = []
                if f < nA:
                    for g in range((n_rg * f) // nA, (n_rg * (f + 1)) // nA):
                        o_parts.append(attn_rows(g * R))
                        new.append(o_parts[-1])
                hl = gate_up(f)
                if dep and last_new:
                    hl[0] = tie(hl[0], last_new)
                last_new = new
                if swp:
                    if pend is not None:
                        d = down(*pend)
                        acc = d if acc is None else [a + t for a, t in zip(acc, d)]
                    pend = (f, hl)
                else:
                    d = down(f, hl)
                    acc = d if acc is None else [a + t for a, t in zip(acc, d)]
            if swp:
                acc = [a + t for a, t in zip(acc, down(*pend))]
            y = _c_full(acc)
            if s is None:
                s = wo_dot(o_parts)
            xr = x_v[pl.ds(r_off, SB), :].astype(f32)
            out_v[pl.ds(r_off, SB), :] = (xr + s * (y * jax.nn.sigmoid(y))).astype(out_v.dtype)
            cp_out(r_off).start()

        cp_x(0).start()
        for i in range(nslab):
            for cp in cp_q(i):
                cp.start()
        for b_ in range(nS):
            if b_ + 1 < nS:
                cp_x(b_ + 1).start()
            for cp in cp_kv(b_):
                cp.start()
        cp_o().start()
        for q_ in range(NQ):
            for cp in cp_ffn(q_):
                cp.start()
        z_ref[...] = jnp.zeros((8, 128), u32)
        z = jnp.zeros((8, HALO, 128), f32)
        k_s[:, 0:HALO, :] = z
        v_s[:, 0:HALO, :] = z
        with scope("x0"):
            cp_x(0).wait()
            layernorm(0)

        def loop_prep(i, c):
            for cp in cp_q(i):
                cp.wait()
            prep_pair(wq_v, 0, qc_v, 0, i)
            return c

        with scope("prep"):
            lax.fori_loop(0, nslab, loop_prep, 0)

        def wrap(name, body):
            def loop(b, c):
                with scope(name):
                    body(b)
                return c
            return loop

        lax.fori_loop(0, nS, wrap("A0", body_a0), 0)
        lax.fori_loop(0, NQ, wrap("A1", body_a1), 0)
        nb = nS if nb_steps is None else nb_steps
        lax.fori_loop(0, nb, wrap("B", body_b), 0)
        with scope("wait_out"):
            for i in range(nb):
                cp_out(i * SB).wait()

    def run(A_x, A_wqkv, A_wo, B_w_gate, B_w_up, B_w_down):
        any_spec = pl.BlockSpec(memory_space=pl.ANY)
        if EMULATE_PACK:
            def pk(w):
                b = lax.bitcast_convert_type(w, jnp.uint16).astype(u32)
                return b[0::2] | (b[1::2] << 16)
            A_wqkv, A_wo, B_w_gate, B_w_up, B_w_down = map(pk, (A_wqkv, A_wo, B_w_gate, B_w_up, B_w_down))
        vm = pltpu.VMEM
        out = pl.pallas_call(
            kernel,
            in_specs=[any_spec] * 6,
            out_specs=any_spec,
            out_shape=jax.ShapeDtypeStruct((S, D), bf16),
            scratch_shapes=[
                vm((S, D), bf16), vm((7, S // 4, DHALF), u32), vm((S, D), bf16),
                vm((DP, D), u32), vm((1, 5, KP, DHALF), u32), vm((DP, 2 * D), u32), vm((2, 5, KP, DHALF), u32),
                vm((DP, D), u32), vm((8, 8 * WOP, 128), u32), vm((5, KP, DHALF), u32),
                vm((DP, F), u32), vm((DP, F), u32), vm((F // 2, D), u32),
                vm((5, KP, F // 2), u32), vm((5, KP, F // 2), u32), vm((5, F // 4, DHALF), u32),
                vm((8, S, 128), f32), vm((8, HALO + S, 128), f32), vm((8, HALO + S, 128), f32), vm((8, 128), u32),
                pltpu.SemaphoreType.DMA((2 + nS + nslab + nS + NQ,)),
            ],
            compiler_params=pltpu.CompilerParams(vmem_limit_bytes=124 << 20, flags=flags),
            name="fused",
            interpret=interpret,
        )(A_x.reshape(S, D), A_wqkv, A_wo, B_w_gate, B_w_up, B_w_down)
        return out.reshape(1, S, D)

    return run


@jax.jit
def pallas_recurrent_scan__sliding_local_dilated__swiglu_ffn__prompt_kernel(
    A_x: jax.Array,
    A_wqkv: jax.Array,
    A_wo: jax.Array,
    B_x: jax.Array,
    B_w_gate: jax.Array,
    B_w_up: jax.Array,
    B_w_down: jax.Array,
):
    del B_x
    return make_kernel(swp=True)(A_x, A_wqkv, A_wo, B_w_gate, B_w_up, B_w_down)
```

```python
import functools
import math

import jax
import jax.numpy as jnp
import numpy as np
from jax import lax
from jax.experimental import pallas as pl
from jax.experimental.pallas import tpu as pltpu

S, D, F = 2048, 1024, 3584
H, DH, WIN, DIL = 32, 32, 8, 2
EPS = 1e-5
HALO = 16
NEG = -1e9
bf16, f32, u32 = jnp.bfloat16, jnp.float32, jnp.uint32
WOP = 65
BFLY = ((1, 2), (2, 4), (4, 8))
DP, DHALF = D // 2, D // 2
KP = D // 4


def _roll(x, s):
    return pltpu.roll(x, s % 128, 1)


def _lanebit_clear(shape, bit):
    return (lax.broadcasted_iota(jnp.int32, shape, 1) & bit) == 0


def _butterfly(t):
    for tb, lb in BFLY:
        msk = _lanebit_clear(t[0].shape, lb)
        n = [None] * 8
        for a in range(8):
            if a & tb:
                continue
            b = a | tb
            n[a] = jnp.where(msk, t[a], _roll(t[b], lb))
            n[b] = jnp.where(msk, _roll(t[a], -lb), t[b])
        t = n
    return t


def _dot(a, b):
    return jnp.dot(a, b, preferred_element_type=f32)


def _a_combos(a):
    m, k = a.shape[0] // 2, a.shape[1] // 2
    a11, a12, a21, a22 = a[:m, :k], a[:m, k:], a[m:, :k], a[m:, k:]
    return [t.astype(bf16) for t in (a11 + a22, a21 + a22, a11, a22, a11 + a12, a21 - a11, a12 - a22)]


def _c_combos(m):
    return (m[0] + m[3] - m[4] + m[6], m[2] + m[4], m[1] + m[3], m[0] - m[1] + m[2] + m[5])


def _c_full(m):
    c11, c12, c21, c22 = _c_combos(m)
    return jnp.concatenate([jnp.concatenate([c11, c12], axis=1), jnp.concatenate([c21, c22], axis=1)], axis=0)


EMULATE_PACK = False


def _unpack(t, i):
    if EMULATE_PACK:
        return lax.bitcast_convert_type((t << 16) if i == 0 else (t & jnp.uint32(0xFFFF0000)), f32)
    return pltpu.unpack_elementwise(t, index=i, packed_dtype=bf16, unpacked_dtype=f32)


def _pack(lo, hi):
    if EMULATE_PACK:
        b = lambda v: lax.bitcast_convert_type(v.astype(bf16).astype(f32), u32)
        return (b(lo) >> 16) | b(hi)
    return pltpu.bitcast(pltpu.pack_elementwise([lo, hi], packed_dtype=bf16), u32)


def _b_combos(b11, b12, b21, b22):
    def half(i):
        return [_unpack(t, i) for t in (b11, b12, b21, b22)]

    def five(x11, x12, x21, x22):
        return (x11 + x22, x12 - x22, x21 - x11, x11 + x12, x21 + x22)

    return [_pack(lo, hi) for lo, hi in zip(five(*half(0)), five(*half(1)))]


def _rhs7(b11, b22, cmb):
    r = [cmb(0), b11, cmb(1), cmb(2), b22, cmb(3), cmb(4)]
    return [pltpu.bitcast(t, bf16) for t in r]


class _Null:
    def __enter__(self):
        return self

    def __exit__(self, *a):
        return False


def make_kernel(SB=256, FC=512, R=8, SBA=512, swp=True, scopes=False, flags=None, nb_steps=None, st_o=True,
                interpret=False, b_frac=0.85, a0_fine=True, b_fine=True, a1_skip=1, a0_skip=0):
    nS = S // SB
    nF = F // FC
    FH = FC // 2
    HB = SB // 2
    XP = HB // 2
    NQ = S // SBA
    GR = KP // NQ
    DC = DHALF // NQ
    slab = KP // 4
    nslab = 4
    assert nS == 2 * nslab and NQ == 4 and DC % 128 == 0 and GR % 8 == 0 and FH % 128 == 0 and (FH // 2) % 8 == 0

    def kernel(x_hbm, wqkv_hbm, wo_hbm, wg_hbm, wu_hbm, wd_hbm, out_hbm,
               x_v, xl_v, out_v, wq_v, qc_v, wkv_v, kvc_v, wo_v, wop, woc,
               wg_v, wu_v, wd_v, gc, uc, dc, q_s, k_s, v_s, o_s, z_ref, sems):
        SEM_OUT, SEM_O = 0, 1
        SEM_X = 2
        SEM_Q = SEM_X + nS
        SEM_KV = SEM_Q + nslab
        SEM_F = SEM_KV + nS

        def scope(name):
            return jax.named_scope(name) if scopes else _Null()

        def w32(ref):
            return ref if EMULATE_PACK else ref.bitcast(u32)

        def mult(v, m):
            return v if isinstance(v, int) else pl.multiple_of(v, m)

        def cp_x(i):
            r0 = mult(i * SB, SB)
            return pltpu.make_async_copy(x_hbm.at[pl.ds(r0, SB)], x_v.at[pl.ds(r0, SB)], sems.at[SEM_X + i])

        def cp_pair(dst, dst_c0, m, i, sem):
            cps = []
            for kh in range(2):
                p0 = mult(kh * KP + i * slab, slab)
                cps.append(pltpu.make_async_copy(
                    w32(wqkv_hbm).at[pl.ds(p0, slab), pl.ds(mult(m * D, D), D)],
                    dst.at[pl.ds(p0, slab), pl.ds(dst_c0, D)], sems.at[sem]))
            return cps

        def cp_q(i):
            return cp_pair(wq_v, 0, 0, i, SEM_Q + i)

        def cp_kv(b):
            m, i = b // nslab, b % nslab
            return cp_pair(wkv_v, mult(m * D, D), 1 + m, i, SEM_KV + b)

        def cp_o():
            return pltpu.make_async_copy(w32(wo_hbm), wo_v, sems.at[SEM_O])

        def cp_ffn(q):
            cps = []
            for src, dst in ((wg_hbm, wg_v), (wu_hbm, wu_v)):
                for kh in range(2):
                    r0 = mult(kh * KP + q * GR, 8)
                    cps.append(pltpu.make_async_copy(w32(src).at[pl.ds(r0, GR), :], dst.at[pl.ds(r0, GR), :], sems.at[SEM_F + q]))
            for nh in range(2):
                c0 = mult(nh * DHALF + q * DC, 128)
                cps.append(pltpu.make_async_copy(w32(wd_hbm).at[:, pl.ds(c0, DC)], wd_v.at[:, pl.ds(c0, DC)], sems.at[SEM_F + q]))
            return cps

        def cp_out(r0):
            return pltpu.make_async_copy(out_v.at[pl.ds(r0, SB)], out_hbm.at[pl.ds(r0, SB)], sems.at[SEM_OUT])

        def tied(v, tie):
            if tie is None:
                return v
            if v.shape[1] > 128:
                return jnp.concatenate([tied(v[:, 0:128], tie), v[:, 128:]], axis=1)
            if v.shape[0] > 8:
                return jnp.concatenate([tied(v[0:8], tie), v[8:]], axis=0)
            return pltpu.bitcast(pltpu.bitcast(v, u32) | tie, v.dtype)

        class Pacer:
            def __init__(self, stages, ndots):
                self.stages, self.ndots, self.k, self.done = list(stages), ndots, 0, 0

            def after_dot(self, m):
                self.k += 1
                target = len(self.stages) if self.k >= self.ndots else (len(self.stages) * self.k) // self.ndots
                n = target - self.done
                if n <= 0:
                    return
                nr, nc = m.shape[0] // 8, m.shape[1] // 128
                zero = z_ref[...]
                for i in range(n):
                    t = (i * nr * nc) // n
                    c, r = t // nr, t % nr
                    self.stages[self.done + i](pltpu.bitcast(m[8 * r:8 * r + 8, 128 * c:128 * (c + 1)], u32) & zero)
                self.done = target

            def flush(self):
                for st in self.stages[self.done:]:
                    st(None)
                self.done = len(self.stages)

        def prep_pair(raw, c0, cmb, mi, i, r0=0, nr=None, tie=None):
            nr = slab if nr is None else nr
            p1 = mult(i * slab, slab) + r0
            p2 = mult(KP + i * slab, slab) + r0
            t1 = [raw[pl.ds(p1, nr), pl.ds(c0 + 128 * j, 128)] for j in range(8)]
            t2 = [raw[pl.ds(p2, nr), pl.ds(c0 + 128 * j, 128)] for j in range(8)]
            t1[0] = tied(t1[0], tie)
            t2[0] = tied(t2[0], tie)
            t1, t2 = _butterfly(t1), _butterfly(t2)
            for j in range(4):
                raw[pl.ds(p1, nr), pl.ds(c0 + 128 * j, 128)] = t1[j]
                raw[pl.ds(p2, nr), pl.ds(c0 + 128 * (4 + j), 128)] = t2[4 + j]
                o = _b_combos(t1[j], t1[4 + j], t2[j], t2[4 + j])
                for k in range(5):
                    cmb[mi, k, pl.ds(p1, nr), 128 * j:128 * (j + 1)] = o[k]

        def qkv_rhs(raw, c0, cmb, mi):
            return _rhs7(raw[0:KP, c0:c0 + DHALF], raw[KP:2 * KP, c0 + DHALF:c0 + D], lambda k: cmb[mi, k])

        def ffn_pieces(q):
            r0 = pl.multiple_of(q * GR, 8)
            c0 = pl.multiple_of(q * DC, 128)
            CR = 8
            out = []

            def gu_piece(raw, dst, f, ct, rr, tie=None):
                cl, cr = f * FC + ct * 128, f * FC + FH + ct * 128
                o = _b_combos(tied(raw[pl.ds(r0 + rr, CR), cl:cl + 128], tie), raw[pl.ds(r0 + rr, CR), cr:cr + 128],
                              raw[pl.ds(KP + r0 + rr, CR), cl:cl + 128], raw[pl.ds(KP + r0 + rr, CR), cr:cr + 128])
                for k in range(5):
                    dst[k, pl.ds(r0 + rr, CR), f * FH + ct * 128:f * FH + (ct + 1) * 128] = o[k]

            def d_piece(f, rr, cc, tie=None):
                k0, kq = f * FH + rr, FH // 2
                o = _b_combos(tied(wd_v[k0:k0 + CR, pl.ds(c0 + cc, 128)], tie), wd_v[k0:k0 + CR, pl.ds(DHALF + c0 + cc, 128)],
                              wd_v[k0 + kq:k0 + kq + CR, pl.ds(c0 + cc, 128)], wd_v[k0 + kq:k0 + kq + CR, pl.ds(DHALF + c0 + cc, 128)])
                for k in range(5):
                    dc[k, f * kq + rr:f * kq + rr + CR, pl.ds(c0 + cc, 128)] = o[k]

            for raw, dst in ((wg_v, gc), (wu_v, uc)):
                for f in range(nF):
                    for ct in range(FH // 128):
                        for rr in range(0, GR, CR):
                            out.append(functools.partial(gu_piece, raw, dst, f, ct, rr))
            for f in range(nF):
                for cc in range(0, DC, 128):
                    for rr in range(0, FH // 2, CR):
                        out.append(functools.partial(d_piece, f, rr, cc))
            return out

        def wo_pieces(q):
            out = []

            def plane(ct, T, tie=None):
                c0 = pl.multiple_of(ct * 128, 128)
                blk = tied(wo_v[64 * T:64 * (T + 1), pl.ds(c0, 128)], tie)
                for c in range(8):
                    wop[ct, pl.ds(8 * c + T, 8, stride=WOP), :] = blk[8 * c:8 * c + 8, :]

            def combo(jj, rr, tie=None):
                c0 = pl.multiple_of(q * 128, 128)
                r1, r2 = WOP * jj + rr, WOP * (4 + jj) + rr
                o = _b_combos(tied(wop[q, r1:r1 + 8, :], tie), wop[4 + q, r1:r1 + 8, :], wop[q, r2:r2 + 8, :], wop[4 + q, r2:r2 + 8, :])
                for k in range(5):
                    woc[k, 64 * jj + rr:64 * jj + rr + 8, pl.ds(c0, 128)] = o[k]

            for T in range(8):
                out.append(functools.partial(plane, q, T))
                out.append(functools.partial(plane, 4 + q, T))
            if st_o:
                for jj in range(4):
                    for rr in range(0, 64, 8):
                        out.append(functools.partial(combo, jj, rr))
            return out

        def wo_tile(j0, j1, c0, c1):
            return jnp.concatenate(
                [jnp.concatenate([wop[ct, WOP * j:WOP * j + 64, :] for ct in range(c0, c1)], axis=1) for j in range(j0, j1)], axis=0)

        def ln_rows(r0, n, tie=None):
            x = tied(x_v[pl.ds(r0, n), :].astype(f32), tie)
            mean = jnp.mean(x, axis=-1, keepdims=True)
            xc = x - mean
            var = jnp.mean(xc * xc, axis=-1, keepdims=True)
            return xc * lax.rsqrt(var + EPS)

        def layernorm(b, u0=0, nu=None, tie=None):
            nu = HB // 16 if nu is None else nu
            r0 = mult(b * SB, SB) + 16 * u0
            xn = jnp.concatenate([ln_rows(r0, 16 * nu, tie), ln_rows(r0 + HB, 16 * nu)], axis=0)
            p0 = mult(b * XP, XP) + 8 * u0
            for k, l in enumerate(_a_combos(xn)):
                xl_v[k, pl.ds(p0, 8 * nu), :] = pltpu.bitcast(l, u32)

        def xl_lhs(p0, n):
            return [pltpu.bitcast(xl_v[k, pl.ds(p0, n), :], bf16) for k in range(7)]

        def store_planes(dst, row0, nblk, m):
            c11, c12, c21, c22 = _c_combos(m)
            for blk in range(nblk):
                for half, (cl, cr) in enumerate(((c11, c12), (c21, c22))):
                    r = row0 + blk * SB + half * HB
                    for j in range(4):
                        dst[j, pl.ds(r, HB), :] = cl[blk * HB:(blk + 1) * HB, 128 * j:128 * (j + 1)]
                        dst[4 + j, pl.ds(r, HB), :] = cr[blk * HB:(blk + 1) * HB, 128 * j:128 * (j + 1)]

        def body_a0(b):
            @pl.when(b < nS - 1)
            def _():
                cp_x(b + 1).wait()
            for cp in cp_kv(b):
                cp.wait()
            lhs = xl_lhs(pl.multiple_of(b * XP, XP), XP)
            nxt = jnp.minimum(b + 1, nS - 1)

            mi, si = b // nslab, b % nslab
            c0 = pl.multiple_of(mi * D, D)
            if a0_fine:
                stages = []
                for u in range(8):
                    stages.append(lambda tie, u=u: prep_pair(wkv_v, c0, kvc_v, mi, si, 8 * u, 8, tie))
                    stages.append(lambda tie, u=u: layernorm(nxt, u, 1, tie))
                pacer = Pacer(stages, 7 - a0_skip)
            else:
                pacer = Pacer([], 1)
            m = []
            for l, w in zip(lhs, qkv_rhs(wq_v, 0, qc_v, 0)):
                m.append(_dot(l, w))
                pacer.after_dot(m[-1])
            pacer.flush()
            store_planes(q_s, pl.multiple_of(b * SB, SB), 1, m)
            if not a0_fine:
                layernorm(nxt)
                prep_pair(wkv_v, c0, kvc_v, mi, si)

        def body_a1(b):
            @pl.when(b == 0)
            def _():
                cp_o().wait()
            for cp in cp_ffn(b):
                cp.wait()
            nblk = SBA // SB
            lhs = xl_lhs(pl.multiple_of(b * nblk * XP, XP), nblk * XP)
            fp = ffn_pieces(b)
            pacer = Pacer(fp[:40] + wo_pieces(b) + fp[40:], 14 - a1_skip)
            row0 = pl.multiple_of(b * SBA, SBA) + HALO
            for mi, dst in enumerate((k_s, v_s)):
                m = []
                for l, w in zip(lhs, qkv_rhs(wkv_v, mi * D, kvc_v, mi)):
                    m.append(_dot(l, w))
                    pacer.after_dot(m[-1])
                store_planes(dst, row0, nblk, m)
            pacer.flush()

        shp = (R, 128)
        CEXP = (DH ** -0.5) * math.log2(math.e)

        def body_b(b):
            r_off = pl.multiple_of(b * SB, SB)
            m16 = _lanebit_clear(shp, 16)
            m1 = _lanebit_clear(shp, 1)
            xl = xl_lhs(pl.multiple_of(b * XP, XP), XP)

            def swap(z, msk, s):
                return jnp.where(msk, _roll(z, -s), _roll(z, s))

            def merge(a, b_, msk, s):
                return jnp.where(msk, a + _roll(a, -s), b_ + _roll(b_, s))

            def tree_sum(ts):
                while len(ts) > 1:
                    ts = [ts[i] + ts[i + 1] for i in range(0, len(ts), 2)]
                return ts[0]

            def attn_rows(r0):
                q = None
                P = []
                for w in range(WIN):
                    tie = yield
                    if q is None:
                        q = [q_s[j, pl.ds(r_off + r0, R), :] for j in range(8)]
                    base = r_off + (HALO + r0 - DIL * w)
                    kk = [k_s[j, pl.ds(base, R), :] for j in range(8)]
                    kk[0] = tied(kk[0], tie)
                    P.append(tree_sum([q[j] * kk[j] for j in range(8)]))
                z0 = merge(merge(P[0], P[1], m16, 16), merge(P[2], P[3], m16, 16), m1, 1)
                z1 = merge(merge(P[4], P[5], m16, 16), merge(P[6], P[7], m16, 16), m1, 1)
                if r0 < DIL * (WIN - 1):
                    lane = lax.broadcasted_iota(jnp.int32, shp, 1)
                    row = lax.broadcasted_iota(jnp.int32, shp, 0) + (r0 + r_off)
                    w0 = ((lane >> 4) & 1) + 2 * (lane & 1)
                    z0 = jnp.where(row >= DIL * w0, z0, NEG / (DH ** -0.5))
                    z1 = jnp.where(row >= DIL * (w0 + 4), z1, NEG / (DH ** -0.5))
                mx = jnp.maximum(z0, z1)
                mx = jnp.maximum(mx, swap(mx, m16, 16))
                mx = jnp.maximum(mx, swap(mx, m1, 1))
                e0 = jnp.exp2((z0 - mx) * CEXP)
                e1 = jnp.exp2((z1 - mx) * CEXP)
                den = e0 + e1
                den = den + swap(den, m16, 16)
                den = den + swap(den, m1, 1)
                r = 1.0 / den
                a = []
                for e in (e0 * r, e1 * r):
                    u0 = jnp.where(m1, e, _roll(e, 1))
                    u1 = jnp.where(m1, _roll(e, -1), e)
                    for u in (u0, u1):
                        a.append(jnp.where(m16, u, _roll(u, 16)))
                        a.append(jnp.where(m16, _roll(u, -16), u))
                for j in range(8):
                    tie = yield
                    vv = [v_s[j, pl.ds(r_off + (HALO + r0 - DIL * w), R), :] for w in range(WIN)]
                    vv[0] = tied(vv[0], tie)
                    o_s[r0:r0 + R, 128 * j:128 * (j + 1)] = tree_sum([a[w] * vv[w] for w in range(WIN)])
                yield

            def gu_rhs(raw, cmb, f):
                return _rhs7(raw[0:KP, f * FC:f * FC + FH], raw[KP:2 * KP, f * FC + FH:(f + 1) * FC],
                             lambda k: cmb[k, :, f * FH:(f + 1) * FH])

            def d_rhs(f):
                k0, kq = f * FH, FH // 2
                return _rhs7(wd_v[k0:k0 + kq, 0:DHALF], wd_v[k0 + kq:k0 + 2 * kq, DHALF:D], lambda k: dc[k, f * kq:(f + 1) * kq, :])

            stages = []
            for g in range(SB // R):
                gen = attn_rows(g * R)
                next(gen)
                stages += [gen.send] * (2 * WIN)
            ndots = 21 * nF
            pacer = Pacer(stages, int(ndots * b_frac))

            def pdot(l, w):
                m = _dot(l, w)
                if b_fine:
                    pacer.after_dot(m)
                return m

            if not b_fine:
                pacer.flush()

            def gate_up(f):
                gt = _c_full([pdot(l, w) for l, w in zip(xl, gu_rhs(wg_v, gc, f))])
                up = _c_full([pdot(l, w) for l, w in zip(xl, gu_rhs(wu_v, uc, f))])
                return _a_combos(gt * jax.nn.sigmoid(gt) * up)

            def down(f, hl):
                return [pdot(l, w) for l, w in zip(hl, d_rhs(f))]

            def wo_dot():
                pacer.flush()
                o = o_s[...]
                if st_o:
                    rhs = _rhs7(wo_tile(0, 4, 0, 4), wo_tile(4, 8, 4, 8), lambda k: woc[k])
                    return _c_full([_dot(l, w) for l, w in zip(_a_combos(o), rhs)])
                return _dot(o.astype(bf16), pltpu.bitcast(wo_tile(0, 8, 0, 8), bf16))

            acc, pend = None, None
            for f in range(nF):
                hl = gate_up(f)
                if swp:
                    if pend is not None:
                        d = down(*pend)
                        acc = d if acc is None else [a + t for a, t in zip(acc, d)]
                    pend = (f, hl)
                else:
                    d = down(f, hl)
                    acc = d if acc is None else [a + t for a, t in zip(acc, d)]
            if swp:
                acc = [a + t for a, t in zip(acc, down(*pend))]
            y = _c_full(acc)
            s = wo_dot()
            xr = x_v[pl.ds(r_off, SB), :].astype(f32)
            out_v[pl.ds(r_off, SB), :] = (xr + s * (y * jax.nn.sigmoid(y))).astype(out_v.dtype)
            cp_out(r_off).start()

        cp_x(0).start()
        for i in range(nslab):
            for cp in cp_q(i):
                cp.start()
        for b_ in range(nS):
            if b_ + 1 < nS:
                cp_x(b_ + 1).start()
            for cp in cp_kv(b_):
                cp.start()
        cp_o().start()
        for q_ in range(NQ):
            for cp in cp_ffn(q_):
                cp.start()
        z_ref[...] = jnp.zeros((8, 128), u32)
        z = jnp.zeros((8, HALO, 128), f32)
        k_s[:, 0:HALO, :] = z
        v_s[:, 0:HALO, :] = z
        with scope("x0"):
            cp_x(0).wait()
            layernorm(0)

        def loop_prep(i, c):
            for cp in cp_q(i):
                cp.wait()
            prep_pair(wq_v, 0, qc_v, 0, i)
            return c

        with scope("prep"):
            lax.fori_loop(0, nslab, loop_prep, 0)

        def wrap(name, body):
            def loop(b, c):
                with scope(name):
                    body(b)
                return c
            return loop

        lax.fori_loop(0, nS, wrap("A0", body_a0), 0)
        lax.fori_loop(0, NQ, wrap("A1", body_a1), 0)
        nb = nS if nb_steps is None else nb_steps
        lax.fori_loop(0, nb, wrap("B", body_b), 0)
        with scope("wait_out"):
            for i in range(nb):
                cp_out(i * SB).wait()

    def run(A_x, A_wqkv, A_wo, B_w_gate, B_w_up, B_w_down):
        any_spec = pl.BlockSpec(memory_space=pl.ANY)
        if EMULATE_PACK:
            def pk(w):
                b = lax.bitcast_convert_type(w, jnp.uint16).astype(u32)
                return b[0::2] | (b[1::2] << 16)
            A_wqkv, A_wo, B_w_gate, B_w_up, B_w_down = map(pk, (A_wqkv, A_wo, B_w_gate, B_w_up, B_w_down))
        vm = pltpu.VMEM
        out = pl.pallas_call(
            kernel,
            in_specs=[any_spec] * 6,
            out_specs=any_spec,
            out_shape=jax.ShapeDtypeStruct((S, D), bf16),
            scratch_shapes=[
                vm((S, D), bf16), vm((7, S // 4, DHALF), u32), vm((S, D), bf16),
                vm((DP, D), u32), vm((1, 5, KP, DHALF), u32), vm((DP, 2 * D), u32), vm((2, 5, KP, DHALF), u32),
                vm((DP, D), u32), vm((8, 8 * WOP, 128), u32), vm((5, KP, DHALF), u32),
                vm((DP, F), u32), vm((DP, F), u32), vm((F // 2, D), u32),
                vm((5, KP, F // 2), u32), vm((5, KP, F // 2), u32), vm((5, F // 4, DHALF), u32),
                vm((8, S, 128), f32), vm((8, HALO + S, 128), f32), vm((8, HALO + S, 128), f32), vm((SB, D), f32), vm((8, 128), u32),
                pltpu.SemaphoreType.DMA((2 + nS + nslab + nS + NQ,)),
            ],
            compiler_params=pltpu.CompilerParams(vmem_limit_bytes=124 << 20, flags=flags),
            name="fused",
            interpret=interpret,
        )(A_x.reshape(S, D), A_wqkv, A_wo, B_w_gate, B_w_up, B_w_down)
        return out.reshape(1, S, D)

    return run


@jax.jit
def pallas_recurrent_scan__sliding_local_dilated__swiglu_ffn__prompt_kernel(
    A_x: jax.Array,
    A_wqkv: jax.Array,
    A_wo: jax.Array,
    B_x: jax.Array,
    B_w_gate: jax.Array,
    B_w_up: jax.Array,
    B_w_down: jax.Array,
):
    del B_x
    return make_kernel(a0_skip=1)(A_x, A_wqkv, A_wo, B_w_gate, B_w_up, B_w_down)
```

```python
import functools
import math

import jax
import jax.numpy as jnp
import numpy as np
from jax import lax
from jax.experimental import pallas as pl
from jax.experimental.pallas import tpu as pltpu

S, D, F = 2048, 1024, 3584
H, DH, WIN, DIL = 32, 32, 8, 2
EPS = 1e-5
HALO = 16
NEG = -1e9
bf16, f32, u32 = jnp.bfloat16, jnp.float32, jnp.uint32
WOP = 65
BFLY = ((1, 2), (2, 4), (4, 8))
DP, DHALF = D // 2, D // 2
KP = D // 4


def _roll(x, s):
    return pltpu.roll(x, s % 128, 1)


def _lanebit_clear(shape, bit):
    return (lax.broadcasted_iota(jnp.int32, shape, 1) & bit) == 0


def _butterfly(t):
    for tb, lb in BFLY:
        msk = _lanebit_clear(t[0].shape, lb)
        n = [None] * 8
        for a in range(8):
            if a & tb:
                continue
            b = a | tb
            n[a] = jnp.where(msk, t[a], _roll(t[b], lb))
            n[b] = jnp.where(msk, _roll(t[a], -lb), t[b])
        t = n
    return t


def _dot(a, b):
    return jnp.dot(a, b, preferred_element_type=f32)


def _a_combos(a):
    m, k = a.shape[0] // 2, a.shape[1] // 2
    a11, a12, a21, a22 = a[:m, :k], a[:m, k:], a[m:, :k], a[m:, k:]
    return [t.astype(bf16) for t in (a11 + a22, a21 + a22, a11, a22, a11 + a12, a21 - a11, a12 - a22)]


def _c_combos(m):
    return (m[0] + m[3] - m[4] + m[6], m[2] + m[4], m[1] + m[3], m[0] - m[1] + m[2] + m[5])


def _c_full(m):
    c11, c12, c21, c22 = _c_combos(m)
    return jnp.concatenate([jnp.concatenate([c11, c12], axis=1), jnp.concatenate([c21, c22], axis=1)], axis=0)


EMULATE_PACK = False


def _unpack(t, i):
    if EMULATE_PACK:
        return lax.bitcast_convert_type((t << 16) if i == 0 else (t & jnp.uint32(0xFFFF0000)), f32)
    return pltpu.unpack_elementwise(t, index=i, packed_dtype=bf16, unpacked_dtype=f32)


def _pack(lo, hi):
    if EMULATE_PACK:
        b = lambda v: lax.bitcast_convert_type(v.astype(bf16).astype(f32), u32)
        return (b(lo) >> 16) | b(hi)
    return pltpu.bitcast(pltpu.pack_elementwise([lo, hi], packed_dtype=bf16), u32)


def _b_combos(b11, b12, b21, b22):
    def half(i):
        return [_unpack(t, i) for t in (b11, b12, b21, b22)]

    def five(x11, x12, x21, x22):
        return (x11 + x22, x12 - x22, x21 - x11, x11 + x12, x21 + x22)

    return [_pack(lo, hi) for lo, hi in zip(five(*half(0)), five(*half(1)))]


def _rhs7(b11, b22, cmb):
    r = [cmb(0), b11, cmb(1), cmb(2), b22, cmb(3), cmb(4)]
    return [pltpu.bitcast(t, bf16) for t in r]


class _Null:
    def __enter__(self):
        return self

    def __exit__(self, *a):
        return False


def make_kernel(SB=256, FC=512, R=8, SBA=512, swp=True, scopes=False, flags=None, nb_steps=None, st_o=True,
                interpret=False, b_frac=0.85, a0_fine=True, b_fine=True, a1_skip=1, a0_skip=1, wo_at=7, o_stage=True, nslab0=4):
    nS = S // SB
    nF = F // FC
    FH = FC // 2
    HB = SB // 2
    XP = HB // 2
    NQ = S // SBA
    GR = KP // NQ
    DC = DHALF // NQ
    slab = KP // 4
    nslab = 4
    assert nS == 2 * nslab and NQ == 4 and DC % 128 == 0 and GR % 8 == 0 and FH % 128 == 0 and (FH // 2) % 8 == 0

    def kernel(x_hbm, wqkv_hbm, wo_hbm, wg_hbm, wu_hbm, wd_hbm, out_hbm,
               x_v, xl_v, out_v, wq_v, qc_v, wk_v, kc_v, wv_v, vc_v, wo_v, wop, woc,
               wg_v, wu_v, wd_v, gc, uc, dc, q_s, k_s, v_s, o_s, ol_s, z_ref, sems):
        SEM_OUT, SEM_O = 0, 1
        kslab = KP // nS
        SEM_X = 2
        SEM_Q = SEM_X + nS
        SEM_K = SEM_Q + nslab
        SEM_V = SEM_K + nS
        SEM_G = SEM_V + nslab
        SEM_D = SEM_G + NQ

        def scope(name):
            return jax.named_scope(name) if scopes else _Null()

        def w32(ref):
            return ref if EMULATE_PACK else ref.bitcast(u32)

        def mult(v, m):
            return v if isinstance(v, int) else pl.multiple_of(v, m)

        def cp_x(i):
            r0 = mult(i * SB, SB)
            return pltpu.make_async_copy(x_hbm.at[pl.ds(r0, SB)], x_v.at[pl.ds(r0, SB)], sems.at[SEM_X + i])

        def cp_pair(dst, m, p0, nr, sem):
            cps = []
            for kh in range(2):
                p = mult(kh * KP + p0, nr)
                cps.append(pltpu.make_async_copy(w32(wqkv_hbm).at[pl.ds(p, nr), pl.ds(m * D, D)], dst.at[pl.ds(p, nr), :], sems.at[sem]))
            return cps

        def cp_q(i):
            return cp_pair(wq_v, 0, i * slab, slab, SEM_Q + i)

        def cp_k(b):
            return cp_pair(wk_v, 1, b * kslab, kslab, SEM_K + b)

        def cp_v(i):
            return cp_pair(wv_v, 2, i * slab, slab, SEM_V + i)

        def cp_o():
            return pltpu.make_async_copy(w32(wo_hbm), wo_v, sems.at[SEM_O])

        def cp_gu(q):
            cps = []
            for src, dst in ((wg_hbm, wg_v), (wu_hbm, wu_v)):
                for kh in range(2):
                    r0 = mult(kh * KP + q * GR, 8)
                    cps.append(pltpu.make_async_copy(w32(src).at[pl.ds(r0, GR), :], dst.at[pl.ds(r0, GR), :], sems.at[SEM_G + q]))
            return cps

        def cp_d(q):
            cps = []
            for nh in range(2):
                c0 = mult(nh * DHALF + q * DC, 128)
                cps.append(pltpu.make_async_copy(w32(wd_hbm).at[:, pl.ds(c0, DC)], wd_v.at[:, pl.ds(c0, DC)], sems.at[SEM_D + q]))
            return cps

        def cp_out(r0):
            return pltpu.make_async_copy(out_v.at[pl.ds(r0, SB)], out_hbm.at[pl.ds(r0, SB)], sems.at[SEM_OUT])

        def tied(v, tie):
            if tie is None:
                return v
            if v.shape[1] > 128:
                return jnp.concatenate([tied(v[:, 0:128], tie), v[:, 128:]], axis=1)
            if v.shape[0] > 8:
                return jnp.concatenate([tied(v[0:8], tie), v[8:]], axis=0)
            return pltpu.bitcast(pltpu.bitcast(v, u32) | tie, v.dtype)

        class Pacer:
            def __init__(self, stages, ndots):
                self.stages, self.ndots, self.k, self.done = list(stages), ndots, 0, 0

            def after_dot(self, m):
                self.k += 1
                target = len(self.stages) if self.k >= self.ndots else (len(self.stages) * self.k) // self.ndots
                n = target - self.done
                if n <= 0:
                    return
                nr, nc = m.shape[0] // 8, m.shape[1] // 128
                zero = z_ref[...]
                for i in range(n):
                    t = (i * nr * nc) // n
                    c, r = t // nr, t % nr
                    self.stages[self.done + i](pltpu.bitcast(m[8 * r:8 * r + 8, 128 * c:128 * (c + 1)], u32) & zero)
                self.done = target

            def flush(self):
                for st in self.stages[self.done:]:
                    st(None)
                self.done = len(self.stages)

        def prep_pair(raw, cmb, p0, nr, tie=None):
            p1, p2 = p0, KP + p0
            t1 = [raw[pl.ds(p1, nr), 128 * j:128 * (j + 1)] for j in range(8)]
            t2 = [raw[pl.ds(p2, nr), 128 * j:128 * (j + 1)] for j in range(8)]
            t1[0] = tied(t1[0], tie)
            t2[0] = tied(t2[0], tie)
            t1, t2 = _butterfly(t1), _butterfly(t2)
            for j in range(4):
                raw[pl.ds(p1, nr), 128 * j:128 * (j + 1)] = t1[j]
                raw[pl.ds(p2, nr), 128 * (4 + j):128 * (5 + j)] = t2[4 + j]
                o = _b_combos(t1[j], t1[4 + j], t2[j], t2[4 + j])
                for k in range(5):
                    cmb[0, k, pl.ds(p1, nr), 128 * j:128 * (j + 1)] = o[k]

        def qkv_rhs(raw, cmb):
            return _rhs7(raw[0:KP, 0:DHALF], raw[KP:2 * KP, DHALF:D], lambda k: cmb[0, k])

        def ffn_pieces(q):
            r0 = pl.multiple_of(q * GR, 8)
            c0 = pl.multiple_of(q * DC, 128)
            CR = 8
            out = []

            def gu_piece(raw, dst, f, ct, rr, tie=None):
                cl, cr = f * FC + ct * 128, f * FC + FH + ct * 128
                o = _b_combos(tied(raw[pl.ds(r0 + rr, CR), cl:cl + 128], tie), raw[pl.ds(r0 + rr, CR), cr:cr + 128],
                              raw[pl.ds(KP + r0 + rr, CR), cl:cl + 128], raw[pl.ds(KP + r0 + rr, CR), cr:cr + 128])
                for k in range(5):
                    dst[k, pl.ds(r0 + rr, CR), f * FH + ct * 128:f * FH + (ct + 1) * 128] = o[k]

            def d_piece(f, rr, cc, tie=None):
                k0, kq = f * FH + rr, FH // 2
                o = _b_combos(tied(wd_v[k0:k0 + CR, pl.ds(c0 + cc, 128)], tie), wd_v[k0:k0 + CR, pl.ds(DHALF + c0 + cc, 128)],
                              wd_v[k0 + kq:k0 + kq + CR, pl.ds(c0 + cc, 128)], wd_v[k0 + kq:k0 + kq + CR, pl.ds(DHALF + c0 + cc, 128)])
                for k in range(5):
                    dc[k, f * kq + rr:f * kq + rr + CR, pl.ds(c0 + cc, 128)] = o[k]

            for raw, dst in ((wg_v, gc), (wu_v, uc)):
                for f in range(nF):
                    for ct in range(FH // 128):
                        for rr in range(0, GR, CR):
                            out.append(functools.partial(gu_piece, raw, dst, f, ct, rr))
            out_d = []
            for f in range(nF):
                for cc in range(0, DC, 128):
                    for rr in range(0, FH // 2, CR):
                        out_d.append(functools.partial(d_piece, f, rr, cc))
            return out, out_d

        def wo_pieces(q):
            out = []

            def plane(ct, T, tie=None):
                c0 = pl.multiple_of(ct * 128, 128)
                blk = tied(wo_v[64 * T:64 * (T + 1), pl.ds(c0, 128)], tie)
                for c in range(8):
                    wop[ct, pl.ds(8 * c + T, 8, stride=WOP), :] = blk[8 * c:8 * c + 8, :]

            def combo(jj, rr, tie=None):
                c0 = pl.multiple_of(q * 128, 128)
                r1, r2 = WOP * jj + rr, WOP * (4 + jj) + rr
                o = _b_combos(tied(wop[q, r1:r1 + 8, :], tie), wop[4 + q, r1:r1 + 8, :], wop[q, r2:r2 + 8, :], wop[4 + q, r2:r2 + 8, :])
                for k in range(5):
                    woc[k, 64 * jj + rr:64 * jj + rr + 8, pl.ds(c0, 128)] = o[k]

            for T in range(8):
                out.append(functools.partial(plane, q, T))
                out.append(functools.partial(plane, 4 + q, T))
            if st_o:
                for jj in range(4):
                    for rr in range(0, 64, 8):
                        out.append(functools.partial(combo, jj, rr))
            return out

        def wo_tile(j0, j1, c0, c1):
            return jnp.concatenate(
                [jnp.concatenate([wop[ct, WOP * j:WOP * j + 64, :] for ct in range(c0, c1)], axis=1) for j in range(j0, j1)], axis=0)

        def ln_rows(r0, n, tie=None):
            x = tied(x_v[pl.ds(r0, n), :].astype(f32), tie)
            mean = jnp.mean(x, axis=-1, keepdims=True)
            xc = x - mean
            var = jnp.mean(xc * xc, axis=-1, keepdims=True)
            return xc * lax.rsqrt(var + EPS)

        def layernorm(b, u0=0, nu=None, tie=None):
            nu = HB // 16 if nu is None else nu
            r0 = mult(b * SB, SB) + 16 * u0
            xn = jnp.concatenate([ln_rows(r0, 16 * nu, tie), ln_rows(r0 + HB, 16 * nu)], axis=0)
            p0 = mult(b * XP, XP) + 8 * u0
            for k, l in enumerate(_a_combos(xn)):
                xl_v[k, pl.ds(p0, 8 * nu), :] = pltpu.bitcast(l, u32)

        def xl_lhs(p0, n):
            return [pltpu.bitcast(xl_v[k, pl.ds(p0, n), :], bf16) for k in range(7)]

        def store_planes(dst, row0, nblk, m):
            c11, c12, c21, c22 = _c_combos(m)
            for blk in range(nblk):
                for half, (cl, cr) in enumerate(((c11, c12), (c21, c22))):
                    r = row0 + blk * SB + half * HB
                    for j in range(4):
                        dst[j, pl.ds(r, HB), :] = cl[blk * HB:(blk + 1) * HB, 128 * j:128 * (j + 1)]
                        dst[4 + j, pl.ds(r, HB), :] = cr[blk * HB:(blk + 1) * HB, 128 * j:128 * (j + 1)]

        def body_a0(b):
            @pl.when(b < nS - 1)
            def _():
                cp_x(b + 1).wait()
            for cp in cp_k(b):
                cp.wait()
            lhs = xl_lhs(pl.multiple_of(b * XP, XP), XP)
            nxt = jnp.minimum(b + 1, nS - 1)

            p0 = pl.multiple_of(b * kslab, kslab)
            if a0_fine:
                stages = []
                for u in range(8):
                    if u % 2 == 0:
                        stages.append(lambda tie, u=u: prep_pair(wk_v, kc_v, p0 + 4 * u, 8, tie))
                    stages.append(lambda tie, u=u: layernorm(nxt, u, 1, tie))
                pacer = Pacer(stages, 7 - a0_skip)
            else:
                pacer = Pacer([], 1)
            m = []
            for l, w in zip(lhs, qkv_rhs(wq_v, qc_v)):
                m.append(_dot(l, w))
                pacer.after_dot(m[-1])
            pacer.flush()
            store_planes(q_s, pl.multiple_of(b * SB, SB), 1, m)
            if not a0_fine:
                layernorm(nxt)
                prep_pair(wk_v, kc_v, p0, kslab)

        def kv_proj(b, raw, cmb, dst, stages):
            nblk = SBA // SB
            lhs = xl_lhs(pl.multiple_of(b * nblk * XP, XP), nblk * XP)
            pacer = Pacer(stages, 7 - a1_skip)
            m = []
            for l, w in zip(lhs, qkv_rhs(raw, cmb)):
                m.append(_dot(l, w))
                pacer.after_dot(m[-1])
            store_planes(dst, pl.multiple_of(b * SBA, SBA) + HALO, nblk, m)
            pacer.flush()

        def body_ak(b):
            for cp in cp_v(b) + cp_gu(b):
                cp.wait()
            p0 = pl.multiple_of(b * slab, slab)
            vst = [functools.partial(lambda u, tie: prep_pair(wv_v, vc_v, p0 + 8 * u, 8, tie), u) for u in range(slab // 8)]
            gu = ffn_pieces(b)[0]
            stages = []
            for i, st in enumerate(gu):
                if i % (len(gu) // len(vst)) == 0 and vst:
                    stages.append(vst.pop(0))
                stages.append(st)
            kv_proj(b, wk_v, kc_v, k_s, stages + vst)

        def body_av(b):
            @pl.when(b == 0)
            def _():
                cp_o().wait()
            for cp in cp_d(b):
                cp.wait()
            kv_proj(b, wv_v, vc_v, v_s, wo_pieces(b) + ffn_pieces(b)[1])

        shp = (R, 128)
        CEXP = (DH ** -0.5) * math.log2(math.e)

        def body_b(b):
            r_off = pl.multiple_of(b * SB, SB)
            m16 = _lanebit_clear(shp, 16)
            m1 = _lanebit_clear(shp, 1)
            xl = xl_lhs(pl.multiple_of(b * XP, XP), XP)

            def swap(z, msk, s):
                return jnp.where(msk, _roll(z, -s), _roll(z, s))

            def merge(a, b_, msk, s):
                return jnp.where(msk, a + _roll(a, -s), b_ + _roll(b_, s))

            def tree_sum(ts):
                while len(ts) > 1:
                    ts = [ts[i] + ts[i + 1] for i in range(0, len(ts), 2)]
                return ts[0]

            def attn_rows(r0):
                q = None
                P = []
                for w in range(WIN):
                    tie = yield
                    if q is None:
                        q = [q_s[j, pl.ds(r_off + r0, R), :] for j in range(8)]
                    base = r_off + (HALO + r0 - DIL * w)
                    kk = [k_s[j, pl.ds(base, R), :] for j in range(8)]
                    kk[0] = tied(kk[0], tie)
                    P.append(tree_sum([q[j] * kk[j] for j in range(8)]))
                z0 = merge(merge(P[0], P[1], m16, 16), merge(P[2], P[3], m16, 16), m1, 1)
                z1 = merge(merge(P[4], P[5], m16, 16), merge(P[6], P[7], m16, 16), m1, 1)
                if r0 < DIL * (WIN - 1):
                    lane = lax.broadcasted_iota(jnp.int32, shp, 1)
                    row = lax.broadcasted_iota(jnp.int32, shp, 0) + (r0 + r_off)
                    w0 = ((lane >> 4) & 1) + 2 * (lane & 1)
                    z0 = jnp.where(row >= DIL * w0, z0, NEG / (DH ** -0.5))
                    z1 = jnp.where(row >= DIL * (w0 + 4), z1, NEG / (DH ** -0.5))
                mx = jnp.maximum(z0, z1)
                mx = jnp.maximum(mx, swap(mx, m16, 16))
                mx = jnp.maximum(mx, swap(mx, m1, 1))
                e0 = jnp.exp2((z0 - mx) * CEXP)
                e1 = jnp.exp2((z1 - mx) * CEXP)
                den = e0 + e1
                den = den + swap(den, m16, 16)
                den = den + swap(den, m1, 1)
                r = 1.0 / den
                a = []
                for e in (e0 * r, e1 * r):
                    u0 = jnp.where(m1, e, _roll(e, 1))
                    u1 = jnp.where(m1, _roll(e, -1), e)
                    for u in (u0, u1):
                        a.append(jnp.where(m16, u, _roll(u, 16)))
                        a.append(jnp.where(m16, _roll(u, -16), u))
                for j in range(8):
                    tie = yield
                    vv = [v_s[j, pl.ds(r_off + (HALO + r0 - DIL * w), R), :] for w in range(WIN)]
                    vv[0] = tied(vv[0], tie)
                    o_s[r0:r0 + R, 128 * j:128 * (j + 1)] = tree_sum([a[w] * vv[w] for w in range(WIN)])
                yield

            def gu_rhs(raw, cmb, f):
                return _rhs7(raw[0:KP, f * FC:f * FC + FH], raw[KP:2 * KP, f * FC + FH:(f + 1) * FC],
                             lambda k: cmb[k, :, f * FH:(f + 1) * FH])

            def d_rhs(f):
                k0, kq = f * FH, FH // 2
                return _rhs7(wd_v[k0:k0 + kq, 0:DHALF], wd_v[k0 + kq:k0 + 2 * kq, DHALF:D], lambda k: dc[k, f * kq:(f + 1) * kq, :])

            def o_combos(u, tie):
                top = tied(o_s[16 * u:16 * u + 16, :], tie)
                o = jnp.concatenate([top, o_s[HB + 16 * u:HB + 16 * u + 16, :]], axis=0)
                for k, l in enumerate(_a_combos(o)):
                    ol_s[k, 8 * u:8 * u + 8, :] = pltpu.bitcast(l, u32)

            stages = []
            for u in range(HB // 16):
                for g0 in (16 * u, HB + 16 * u):
                    for r0 in range(g0, g0 + 16, R):
                        gen = attn_rows(r0)
                        next(gen)
                        stages += [gen.send] * (2 * WIN)
                if st_o and o_stage:
                    stages.append(functools.partial(o_combos, u))
            ndots = 21 * min(nF, wo_at) - (7 if swp else 0)
            pacer = Pacer(stages, int(ndots * b_frac))

            def pdot(l, w):
                m = _dot(l, w)
                if b_fine:
                    pacer.after_dot(m)
                return m

            if not b_fine:
                pacer.flush()

            def gate_up(f):
                gt = _c_full([pdot(l, w) for l, w in zip(xl, gu_rhs(wg_v, gc, f))])
                up = _c_full([pdot(l, w) for l, w in zip(xl, gu_rhs(wu_v, uc, f))])
                return _a_combos(gt * jax.nn.sigmoid(gt) * up)

            def down(f, hl):
                return [pdot(l, w) for l, w in zip(hl, d_rhs(f))]

            def wo_dot():
                pacer.flush()
                if st_o:
                    rhs = _rhs7(wo_tile(0, 4, 0, 4), wo_tile(4, 8, 4, 8), lambda k: woc[k])
                    if o_stage:
                        lhs = [pltpu.bitcast(ol_s[k], bf16) for k in range(7)]
                    else:
                        lhs = _a_combos(o_s[...])
                    return _c_full([_dot(l, w) for l, w in zip(lhs, rhs)])
                return _dot(o_s[...].astype(bf16), pltpu.bitcast(wo_tile(0, 8, 0, 8), bf16))

            acc, pend, s = None, None, None
            for f in range(nF):
                if f == wo_at:
                    s = wo_dot()
                hl = gate_up(f)
                if swp:
                    if pend is not None:
                        d = down(*pend)
                        acc = d if acc is None else [a + t for a, t in zip(acc, d)]
                    pend = (f, hl)
                else:
                    d = down(f, hl)
                    acc = d if acc is None else [a + t for a, t in zip(acc, d)]
            if swp:
                acc = [a + t for a, t in zip(acc, down(*pend))]
            y = _c_full(acc)
            if s is None:
                s = wo_dot()
            xr = x_v[pl.ds(r_off, SB), :].astype(f32)
            out_v[pl.ds(r_off, SB), :] = (xr + s * (y * jax.nn.sigmoid(y))).astype(out_v.dtype)
            cp_out(r_off).start()

        cp_x(0).start()
        for i in range(nslab):
            for cp in cp_q(i):
                cp.start()
        for b_ in range(nS):
            if b_ + 1 < nS:
                cp_x(b_ + 1).start()
            for cp in cp_k(b_):
                cp.start()
        for q_ in range(NQ):
            for cp in cp_v(q_) + cp_gu(q_):
                cp.start()
        cp_o().start()
        for q_ in range(NQ):
            for cp in cp_d(q_):
                cp.start()
        z_ref[...] = jnp.zeros((8, 128), u32)
        z = jnp.zeros((8, HALO, 128), f32)
        k_s[:, 0:HALO, :] = z
        v_s[:, 0:HALO, :] = z
        with scope("x0"):
            cp_x(0).wait()
            layernorm(0)

        def loop_prep(i, c):
            for cp in cp_q(i):
                cp.wait()
            prep_pair(wq_v, qc_v, pl.multiple_of(i * slab, slab), slab)
            return c

        with scope("prep"):
            lax.fori_loop(0, nslab, loop_prep, 0)

        def wrap(name, body):
            def loop(b, c):
                with scope(name):
                    body(b)
                return c
            return loop

        lax.fori_loop(0, nS, wrap("A0", body_a0), 0)
        lax.fori_loop(0, NQ, wrap("AK", body_ak), 0)
        lax.fori_loop(0, NQ, wrap("AV", body_av), 0)
        nb = nS if nb_steps is None else nb_steps
        lax.fori_loop(0, nb, wrap("B", body_b), 0)
        with scope("wait_out"):
            for i in range(nb):
                cp_out(i * SB).wait()

    def run(A_x, A_wqkv, A_wo, B_w_gate, B_w_up, B_w_down):
        any_spec = pl.BlockSpec(memory_space=pl.ANY)
        if EMULATE_PACK:
            def pk(w):
                b = lax.bitcast_convert_type(w, jnp.uint16).astype(u32)
                return b[0::2] | (b[1::2] << 16)
            A_wqkv, A_wo, B_w_gate, B_w_up, B_w_down = map(pk, (A_wqkv, A_wo, B_w_gate, B_w_up, B_w_down))
        vm = pltpu.VMEM
        out = pl.pallas_call(
            kernel,
            in_specs=[any_spec] * 6,
            out_specs=any_spec,
            out_shape=jax.ShapeDtypeStruct((S, D), bf16),
            scratch_shapes=[
                vm((S, D), bf16), vm((7, S // 4, DHALF), u32), vm((S, D), bf16),
                vm((DP, D), u32), vm((1, 5, KP, DHALF), u32), vm((DP, D), u32), vm((1, 5, KP, DHALF), u32),
                vm((DP, D), u32), vm((1, 5, KP, DHALF), u32),
                vm((DP, D), u32), vm((8, 8 * WOP, 128), u32), vm((5, KP, DHALF), u32),
                vm((DP, F), u32), vm((DP, F), u32), vm((F // 2, D), u32),
                vm((5, KP, F // 2), u32), vm((5, KP, F // 2), u32), vm((5, F // 4, DHALF), u32),
                vm((8, S, 128), f32), vm((8, HALO + S, 128), f32), vm((8, HALO + S, 128), f32), vm((SB, D), f32), vm((7, XP, DHALF), u32), vm((8, 128), u32),
                pltpu.SemaphoreType.DMA((2 + nS + nslab + nS + nslab + 2 * NQ,)),
            ],
            compiler_params=pltpu.CompilerParams(vmem_limit_bytes=124 << 20, flags=flags),
            name="fused",
            interpret=interpret,
        )(A_x.reshape(S, D), A_wqkv, A_wo, B_w_gate, B_w_up, B_w_down)
        return out.reshape(1, S, D)

    return run


@jax.jit
def pallas_recurrent_scan__sliding_local_dilated__swiglu_ffn__prompt_kernel(
    A_x: jax.Array,
    A_wqkv: jax.Array,
    A_wo: jax.Array,
    B_x: jax.Array,
    B_w_gate: jax.Array,
    B_w_up: jax.Array,
    B_w_down: jax.Array,
):
    del B_x
    return make_kernel()(A_x, A_wqkv, A_wo, B_w_gate, B_w_up, B_w_down)
```

```python
import functools
import math

import jax
import jax.numpy as jnp
from jax import lax
from jax.experimental import pallas as pl
from jax.experimental.pallas import tpu as pltpu

S, D, F = 2048, 1024, 3584
H, DH, WIN, DIL = 32, 32, 8, 2
EPS = 1e-5
NEG = -1e9
bf16, f32, u32 = jnp.bfloat16, jnp.float32, jnp.uint32

SB = 256
SBA = 512
FC = 512
R = 8
HALO = 16
WOP = 65
BFLY = ((1, 2), (2, 4), (4, 8))

NS, NQ, NF = S // SB, S // SBA, F // FC
DP, DHALF, KP, FH = D // 2, D // 2, D // 4, FC // 2
HB = SB // 2
XP = HB // 2
NSLAB = 4
SLAB = KP // NSLAB
KSLAB = KP // NS
GR = KP // NQ
DC = DHALF // NQ
A0_DOTS, A1_DOTS, B_FRAC = 6, 6, 0.85
assert NQ == NSLAB and DC % 128 == 0 and GR % 8 == 0 and KSLAB % 8 == 0 and FH % 128 == 0 and (FH // 2) % 8 == 0


def _roll(x, s):
    return pltpu.roll(x, s % 128, 1)


def _lanebit_clear(shape, bit):
    return (lax.broadcasted_iota(jnp.int32, shape, 1) & bit) == 0


def _butterfly(t):
    for tb, lb in BFLY:
        msk = _lanebit_clear(t[0].shape, lb)
        n = [None] * 8
        for a in range(8):
            if a & tb:
                continue
            b = a | tb
            n[a] = jnp.where(msk, t[a], _roll(t[b], lb))
            n[b] = jnp.where(msk, _roll(t[a], -lb), t[b])
        t = n
    return t


def _silu(x):
    return x * pl.reciprocal(1.0 + jnp.exp(-x), approx=True)


def _dot(a, b):
    return jnp.dot(a, b, preferred_element_type=f32)


def _unpack(t, i):
    return pltpu.unpack_elementwise(t, index=i, packed_dtype=bf16, unpacked_dtype=f32)


def _pack(lo, hi):
    return pltpu.bitcast(pltpu.pack_elementwise([lo, hi], packed_dtype=bf16), u32)


def _w32(ref):
    return ref.bitcast(u32)


def _a_combos(a):
    m, k = a.shape[0] // 2, a.shape[1] // 2
    a11, a12, a21, a22 = a[:m, :k], a[:m, k:], a[m:, :k], a[m:, k:]
    return [t.astype(bf16) for t in (a11 + a22, a21 + a22, a11, a22, a11 + a12, a21 - a11, a12 - a22)]


def _b_combos(b11, b12, b21, b22):
    def five(x11, x12, x21, x22):
        return (x11 + x22, x12 - x22, x21 - x11, x11 + x12, x21 + x22)

    lo = five(*[_unpack(t, 0) for t in (b11, b12, b21, b22)])
    hi = five(*[_unpack(t, 1) for t in (b11, b12, b21, b22)])
    return [_pack(l, h) for l, h in zip(lo, hi)]


def _rhs7(b11, b22, cmb):
    return [pltpu.bitcast(t, bf16) for t in (cmb(0), b11, cmb(1), cmb(2), b22, cmb(3), cmb(4))]


def _c_combos(m):
    return (m[0] + m[3] - m[4] + m[6], m[2] + m[4], m[1] + m[3], m[0] - m[1] + m[2] + m[5])


def _c_full(m):
    c11, c12, c21, c22 = _c_combos(m)
    return jnp.concatenate([jnp.concatenate([c11, c12], axis=1), jnp.concatenate([c21, c22], axis=1)], axis=0)


def _mult(v, m):
    return v if isinstance(v, int) else pl.multiple_of(v, m)


def _kernel(x_hbm, wqkv_hbm, wo_hbm, wg_hbm, wu_hbm, wd_hbm, out_hbm,
            x_v, xl_v, out_v, wq_v, qc_v, wk_v, kc_v, wv_v, vc_v, wo_v, wop, woc,
            wg_v, wu_v, wd_v, gc, uc, dc, q_s, k_s, v_s, o_s, ol_s, z_ref, sems):
    SEM_OUT, SEM_O = 0, 1
    SEM_X = 2
    SEM_Q = SEM_X + NS
    SEM_K = SEM_Q + NSLAB
    SEM_V = SEM_K + NS
    SEM_G = SEM_V + NSLAB
    SEM_D = SEM_G + NQ

    def cp_x(i):
        r0 = _mult(i * SB, SB)
        return pltpu.make_async_copy(x_hbm.at[pl.ds(r0, SB)], x_v.at[pl.ds(r0, SB)], sems.at[SEM_X + i])

    def cp_pair(dst, m, p0, nr, sem):
        cps = []
        for kh in range(2):
            p = _mult(kh * KP + p0, nr)
            cps.append(pltpu.make_async_copy(
                _w32(wqkv_hbm).at[pl.ds(p, nr), pl.ds(m * D, D)], dst.at[pl.ds(p, nr), :], sems.at[sem]))
        return cps

    def cp_q(i):
        return cp_pair(wq_v, 0, i * SLAB, SLAB, SEM_Q + i)

    def cp_k(b):
        return cp_pair(wk_v, 1, b * KSLAB, KSLAB, SEM_K + b)

    def cp_v(i):
        return cp_pair(wv_v, 2, i * SLAB, SLAB, SEM_V + i)

    def cp_o():
        return pltpu.make_async_copy(_w32(wo_hbm), wo_v, sems.at[SEM_O])

    def cp_gu(q):
        cps = []
        for src, dst in ((wg_hbm, wg_v), (wu_hbm, wu_v)):
            for kh in range(2):
                r0 = _mult(kh * KP + q * GR, 8)
                cps.append(pltpu.make_async_copy(
                    _w32(src).at[pl.ds(r0, GR), :], dst.at[pl.ds(r0, GR), :], sems.at[SEM_G + q]))
        return cps

    def cp_d(q):
        cps = []
        for nh in range(2):
            c0 = _mult(nh * DHALF + q * DC, 128)
            cps.append(pltpu.make_async_copy(
                _w32(wd_hbm).at[:, pl.ds(c0, DC)], wd_v.at[:, pl.ds(c0, DC)], sems.at[SEM_D + q]))
        return cps

    def cp_out(r0):
        return pltpu.make_async_copy(out_v.at[pl.ds(r0, SB)], out_hbm.at[pl.ds(r0, SB)], sems.at[SEM_OUT])

    def tied(v, tie):
        if tie is None:
            return v
        if v.shape[1] > 128:
            return jnp.concatenate([tied(v[:, 0:128], tie), v[:, 128:]], axis=1)
        if v.shape[0] > 8:
            return jnp.concatenate([tied(v[0:8], tie), v[8:]], axis=0)
        return pltpu.bitcast(pltpu.bitcast(v, u32) | tie, v.dtype)

    class Pacer:
        def __init__(self, stages, ndots):
            self.stages, self.ndots, self.k, self.done = list(stages), ndots, 0, 0

        def after_dot(self, m):
            self.k += 1
            total = len(self.stages)
            target = total if self.k >= self.ndots else (total * self.k) // self.ndots
            n = target - self.done
            if n <= 0:
                return
            nr, nc = m.shape[0] // 8, m.shape[1] // 128
            zero = z_ref[...]
            for i in range(n):
                c, r = divmod((i * nr * nc) // n, nr)
                self.stages[self.done + i](pltpu.bitcast(m[8 * r:8 * r + 8, 128 * c:128 * (c + 1)], u32) & zero)
            self.done = target

        def flush(self):
            for st in self.stages[self.done:]:
                st(None)
            self.done = len(self.stages)

    def prep_pair(raw, cmb, p0, nr, tie=None):
        p1, p2 = p0, KP + p0
        t1 = [raw[pl.ds(p1, nr), 128 * j:128 * (j + 1)] for j in range(8)]
        t2 = [raw[pl.ds(p2, nr), 128 * j:128 * (j + 1)] for j in range(8)]
        t1[0] = tied(t1[0], tie)
        t2[0] = tied(t2[0], tie)
        t1, t2 = _butterfly(t1), _butterfly(t2)
        for j in range(4):
            raw[pl.ds(p1, nr), 128 * j:128 * (j + 1)] = t1[j]
            raw[pl.ds(p2, nr), 128 * (4 + j):128 * (5 + j)] = t2[4 + j]
            o = _b_combos(t1[j], t1[4 + j], t2[j], t2[4 + j])
            for k in range(5):
                cmb[k, pl.ds(p1, nr), 128 * j:128 * (j + 1)] = o[k]

    def qkv_rhs(raw, cmb):
        return _rhs7(raw[0:KP, 0:DHALF], raw[KP:2 * KP, DHALF:D], lambda k: cmb[k])

    def gu_pieces(q):
        r0 = pl.multiple_of(q * GR, 8)

        def piece(raw, dst, f, ct, rr, tie=None):
            cl, cr = f * FC + ct * 128, f * FC + FH + ct * 128
            o = _b_combos(tied(raw[pl.ds(r0 + rr, 8), cl:cl + 128], tie), raw[pl.ds(r0 + rr, 8), cr:cr + 128],
                          raw[pl.ds(KP + r0 + rr, 8), cl:cl + 128], raw[pl.ds(KP + r0 + rr, 8), cr:cr + 128])
            for k in range(5):
                dst[k, pl.ds(r0 + rr, 8), f * FH + ct * 128:f * FH + (ct + 1) * 128] = o[k]

        return [functools.partial(piece, raw, dst, f, ct, rr)
                for raw, dst in ((wg_v, gc), (wu_v, uc))
                for f in range(NF) for ct in range(FH // 128) for rr in range(0, GR, 8)]

    def d_pieces(q):
        c0 = pl.multiple_of(q * DC, 128)
        kq = FH // 2

        def piece(f, rr, cc, tie=None):
            k0 = f * FH + rr
            o = _b_combos(tied(wd_v[k0:k0 + 8, pl.ds(c0 + cc, 128)], tie), wd_v[k0:k0 + 8, pl.ds(DHALF + c0 + cc, 128)],
                          wd_v[k0 + kq:k0 + kq + 8, pl.ds(c0 + cc, 128)],
                          wd_v[k0 + kq:k0 + kq + 8, pl.ds(DHALF + c0 + cc, 128)])
            for k in range(5):
                dc[k, f * kq + rr:f * kq + rr + 8, pl.ds(c0 + cc, 128)] = o[k]

        return [functools.partial(piece, f, rr, cc)
                for f in range(NF) for cc in range(0, DC, 128) for rr in range(0, kq, 8)]

    def wo_pieces(q):
        def plane(ct, T, tie=None):
            blk = tied(wo_v[64 * T:64 * (T + 1), pl.ds(pl.multiple_of(ct * 128, 128), 128)], tie)
            for c in range(8):
                wop[ct, pl.ds(8 * c + T, 8, stride=WOP), :] = blk[8 * c:8 * c + 8, :]

        def combo(jj, rr, tie=None):
            r1, r2 = WOP * jj + rr, WOP * (4 + jj) + rr
            o = _b_combos(tied(wop[q, r1:r1 + 8, :], tie), wop[4 + q, r1:r1 + 8, :],
                          wop[q, r2:r2 + 8, :], wop[4 + q, r2:r2 + 8, :])
            for k in range(5):
                woc[k, 64 * jj + rr:64 * jj + rr + 8, pl.ds(pl.multiple_of(q * 128, 128), 128)] = o[k]

        out = [functools.partial(plane, ct, T) for T in range(8) for ct in (q, 4 + q)]
        return out + [functools.partial(combo, jj, rr) for jj in range(4) for rr in range(0, 64, 8)]

    def wo_tile(j0, j1, c0, c1):
        return jnp.concatenate(
            [jnp.concatenate([wop[ct, WOP * j:WOP * j + 64, :] for ct in range(c0, c1)], axis=1) for j in range(j0, j1)],
            axis=0)

    def ln_rows(r0, n, tie=None):
        x = tied(x_v[pl.ds(r0, n), :].astype(f32), tie)
        mean = jnp.mean(x, axis=-1, keepdims=True)
        xc = x - mean
        var = jnp.mean(xc * xc, axis=-1, keepdims=True)
        return xc * lax.rsqrt(var + EPS)

    def layernorm(b, u0=0, nu=HB // 16, tie=None):
        r0 = _mult(b * SB, SB) + 16 * u0
        xn = jnp.concatenate([ln_rows(r0, 16 * nu, tie), ln_rows(r0 + HB, 16 * nu)], axis=0)
        p0 = _mult(b * XP, XP) + 8 * u0
        for k, l in enumerate(_a_combos(xn)):
            xl_v[k, pl.ds(p0, 8 * nu), :] = pltpu.bitcast(l, u32)

    def xl_lhs(p0, n):
        return [pltpu.bitcast(xl_v[k, pl.ds(p0, n), :], bf16) for k in range(7)]

    def store_planes(dst, row0, nblk, m):
        c11, c12, c21, c22 = _c_combos(m)
        for blk in range(nblk):
            for half, (cl, cr) in enumerate(((c11, c12), (c21, c22))):
                r = row0 + blk * SB + half * HB
                for j in range(4):
                    dst[j, pl.ds(r, HB), :] = cl[blk * HB:(blk + 1) * HB, 128 * j:128 * (j + 1)]
                    dst[4 + j, pl.ds(r, HB), :] = cr[blk * HB:(blk + 1) * HB, 128 * j:128 * (j + 1)]

    def paced_product(lhs, rhs, stages, ndots):
        pacer = Pacer(stages, ndots)
        m = []
        for l, w in zip(lhs, rhs):
            m.append(_dot(l, w))
            pacer.after_dot(m[-1])
        pacer.flush()
        return m

    def body_a0(b, carry):
        @pl.when(b < NS - 1)
        def _():
            cp_x(b + 1).wait()
        for cp in cp_k(b):
            cp.wait()
        lhs = xl_lhs(pl.multiple_of(b * XP, XP), XP)
        nxt = jnp.minimum(b + 1, NS - 1)
        p0 = pl.multiple_of(b * KSLAB, KSLAB)
        stages = []
        for u in range(HB // 16):
            if u % 2 == 0:
                stages.append(functools.partial(prep_pair, wk_v, kc_v, p0 + 4 * u, 8))
            stages.append(functools.partial(layernorm, nxt, u, 1))
        m = paced_product(lhs, qkv_rhs(wq_v, qc_v), stages, A0_DOTS)
        store_planes(q_s, pl.multiple_of(b * SB, SB), 1, m)
        return carry

    def kv_proj(b, raw, cmb, dst, stages):
        nblk = SBA // SB
        lhs = xl_lhs(pl.multiple_of(b * nblk * XP, XP), nblk * XP)
        m = paced_product(lhs, qkv_rhs(raw, cmb), stages, A1_DOTS)
        store_planes(dst, pl.multiple_of(b * SBA, SBA) + HALO, nblk, m)

    def body_ak(b, carry):
        for cp in cp_v(b) + cp_gu(b):
            cp.wait()
        p0 = pl.multiple_of(b * SLAB, SLAB)
        vst = [functools.partial(prep_pair, wv_v, vc_v, p0 + 8 * u, 8) for u in range(SLAB // 8)]
        gu = gu_pieces(b)
        every = len(gu) // len(vst)
        stages = []
        for i, st in enumerate(gu):
            if i % every == 0:
                stages.append(vst[i // every])
            stages.append(st)
        kv_proj(b, wk_v, kc_v, k_s, stages)
        return carry

    def body_av(b, carry):
        @pl.when(b == 0)
        def _():
            cp_o().wait()
        for cp in cp_d(b):
            cp.wait()
        kv_proj(b, wv_v, vc_v, v_s, wo_pieces(b) + d_pieces(b))
        return carry

    shp = (R, 128)
    SCALE = DH ** -0.5
    CEXP = SCALE * math.log2(math.e)

    def body_b(b, carry):
        r_off = pl.multiple_of(b * SB, SB)
        m16 = _lanebit_clear(shp, 16)
        m1 = _lanebit_clear(shp, 1)
        xl = xl_lhs(pl.multiple_of(b * XP, XP), XP)

        def swap(z, msk, s):
            return jnp.where(msk, _roll(z, -s), _roll(z, s))

        def merge(p, q, msk, s):
            return jnp.where(msk, p + _roll(p, -s), q + _roll(q, s))

        def tree_sum(ts):
            while len(ts) > 1:
                ts = [ts[i] + ts[i + 1] for i in range(0, len(ts), 2)]
            return ts[0]

        def attn_rows(r0):
            q = None
            P = []
            for w in range(WIN):
                tie = yield
                if q is None:
                    q = [q_s[j, pl.ds(r_off + r0, R), :] for j in range(8)]
                base = r_off + (HALO + r0 - DIL * w)
                kk = [k_s[j, pl.ds(base, R), :] for j in range(8)]
                kk[0] = tied(kk[0], tie)
                P.append(tree_sum([q[j] * kk[j] for j in range(8)]))
            z0 = merge(merge(P[0], P[1], m16, 16), merge(P[2], P[3], m16, 16), m1, 1)
            z1 = merge(merge(P[4], P[5], m16, 16), merge(P[6], P[7], m16, 16), m1, 1)
            if r0 < DIL * (WIN - 1):
                lane = lax.broadcasted_iota(jnp.int32, shp, 1)
                row = lax.broadcasted_iota(jnp.int32, shp, 0) + (r0 + r_off)
                w0 = ((lane >> 4) & 1) + 2 * (lane & 1)
                z0 = jnp.where(row >= DIL * w0, z0, NEG / SCALE)
                z1 = jnp.where(row >= DIL * (w0 + 4), z1, NEG / SCALE)
            mx = jnp.maximum(z0, z1)
            mx = jnp.maximum(mx, swap(mx, m16, 16))
            mx = jnp.maximum(mx, swap(mx, m1, 1))
            e0 = jnp.exp2((z0 - mx) * CEXP)
            e1 = jnp.exp2((z1 - mx) * CEXP)
            den = e0 + e1
            den = den + swap(den, m16, 16)
            den = den + swap(den, m1, 1)
            inv = 1.0 / den
            a = []
            for e in (e0 * inv, e1 * inv):
                u0 = jnp.where(m1, e, _roll(e, 1))
                u1 = jnp.where(m1, _roll(e, -1), e)
                for u in (u0, u1):
                    a.append(jnp.where(m16, u, _roll(u, 16)))
                    a.append(jnp.where(m16, _roll(u, -16), u))
            for j in range(8):
                tie = yield
                vv = [v_s[j, pl.ds(r_off + (HALO + r0 - DIL * w), R), :] for w in range(WIN)]
                vv[0] = tied(vv[0], tie)
                o_s[r0:r0 + R, 128 * j:128 * (j + 1)] = tree_sum([a[w] * vv[w] for w in range(WIN)])
            yield

        def o_combos(u, tie):
            top = tied(o_s[16 * u:16 * u + 16, :], tie)
            o = jnp.concatenate([top, o_s[HB + 16 * u:HB + 16 * u + 16, :]], axis=0)
            for k, l in enumerate(_a_combos(o)):
                ol_s[k, 8 * u:8 * u + 8, :] = pltpu.bitcast(l, u32)

        stages = []
        for u in range(HB // 16):
            for g0 in (16 * u, HB + 16 * u):
                for r0 in range(g0, g0 + 16, R):
                    gen = attn_rows(r0)
                    next(gen)
                    stages += [gen.send] * (2 * WIN)
            stages.append(functools.partial(o_combos, u))
        pacer = Pacer(stages, int((21 * NF - 7) * B_FRAC))

        def pdots(lhs, rhs):
            m = []
            for l, w in zip(lhs, rhs):
                m.append(_dot(l, w))
                pacer.after_dot(m[-1])
            return m

        def gu_rhs(raw, cmb, f):
            return _rhs7(raw[0:KP, f * FC:f * FC + FH], raw[KP:2 * KP, f * FC + FH:(f + 1) * FC],
                         lambda k: cmb[k, :, f * FH:(f + 1) * FH])

        def d_rhs(f):
            k0, kq = f * FH, FH // 2
            return _rhs7(wd_v[k0:k0 + kq, 0:DHALF], wd_v[k0 + kq:k0 + 2 * kq, DHALF:D],
                         lambda k: dc[k, f * kq:(f + 1) * kq, :])

        acc, pend = None, None
        for f in range(NF):
            gt = _c_full(pdots(xl, gu_rhs(wg_v, gc, f)))
            up = _c_full(pdots(xl, gu_rhs(wu_v, uc, f)))
            hl = _a_combos(_silu(gt) * up)
            if pend is not None:
                d = pdots(pend[1], d_rhs(pend[0]))
                acc = d if acc is None else [p + t for p, t in zip(acc, d)]
            pend = (f, hl)
        acc = [p + t for p, t in zip(acc, pdots(pend[1], d_rhs(pend[0])))]
        y = _c_full(acc)
        pacer.flush()
        rhs = _rhs7(wo_tile(0, 4, 0, 4), wo_tile(4, 8, 4, 8), lambda k: woc[k])
        s = _c_full([_dot(pltpu.bitcast(ol_s[k], bf16), rhs[k]) for k in range(7)])
        xr = x_v[pl.ds(r_off, SB), :].astype(f32)
        out_v[pl.ds(r_off, SB), :] = (xr + s * _silu(y)).astype(out_v.dtype)
        cp_out(r_off).start()
        return carry

    cp_x(0).start()
    for i in range(NSLAB):
        for cp in cp_q(i):
            cp.start()
    for b in range(NS):
        if b + 1 < NS:
            cp_x(b + 1).start()
        for cp in cp_k(b):
            cp.start()
    for q in range(NQ):
        for cp in cp_v(q) + cp_gu(q):
            cp.start()
    cp_o().start()
    for q in range(NQ):
        for cp in cp_d(q):
            cp.start()
    z_ref[...] = jnp.zeros((8, 128), u32)
    k_s[:, 0:HALO, :] = jnp.zeros((8, HALO, 128), f32)
    v_s[:, 0:HALO, :] = jnp.zeros((8, HALO, 128), f32)
    cp_x(0).wait()
    layernorm(0)

    def body_prep(i, carry):
        for cp in cp_q(i):
            cp.wait()
        prep_pair(wq_v, qc_v, pl.multiple_of(i * SLAB, SLAB), SLAB)
        return carry

    lax.fori_loop(0, NSLAB, body_prep, 0)
    lax.fori_loop(0, NS, body_a0, 0)
    lax.fori_loop(0, NQ, body_ak, 0)
    lax.fori_loop(0, NQ, body_av, 0)
    lax.fori_loop(0, NS, body_b, 0)
    for i in range(NS):
        cp_out(i * SB).wait()


def _scratch_shapes():
    vm = pltpu.VMEM
    return [
        vm((S, D), bf16), vm((7, S // 4, DHALF), u32), vm((S, D), bf16),
        vm((DP, D), u32), vm((5, KP, DHALF), u32),
        vm((DP, D), u32), vm((5, KP, DHALF), u32),
        vm((DP, D), u32), vm((5, KP, DHALF), u32),
        vm((DP, D), u32), vm((8, 8 * WOP, 128), u32), vm((5, KP, DHALF), u32),
        vm((DP, F), u32), vm((DP, F), u32), vm((F // 2, D), u32),
        vm((5, KP, F // 2), u32), vm((5, KP, F // 2), u32), vm((5, F // 4, DHALF), u32),
        vm((8, S, 128), f32), vm((8, HALO + S, 128), f32), vm((8, HALO + S, 128), f32),
        vm((SB, D), f32), vm((7, XP, DHALF), u32), vm((8, 128), u32),
        pltpu.SemaphoreType.DMA((2 + 2 * NS + 2 * NSLAB + 2 * NQ,)),
    ]


@jax.jit
def pallas_recurrent_scan__sliding_local_dilated__swiglu_ffn__prompt_kernel(
    A_x: jax.Array,
    A_wqkv: jax.Array,
    A_wo: jax.Array,
    B_x: jax.Array,
    B_w_gate: jax.Array,
    B_w_up: jax.Array,
    B_w_down: jax.Array,
):
    del B_x
    assert A_x.shape == (1, S, D) and A_wqkv.shape == (D, 3 * D) and B_w_gate.shape == (D, F)
    any_spec = pl.BlockSpec(memory_space=pl.ANY)
    out = pl.pallas_call(
        _kernel,
        in_specs=[any_spec] * 6,
        out_specs=any_spec,
        out_shape=jax.ShapeDtypeStruct((S, D), bf16),
        scratch_shapes=_scratch_shapes(),
        compiler_params=pltpu.CompilerParams(vmem_limit_bytes=124 << 20),
        name="fused_attn_swiglu",
    )(A_x.reshape(S, D), A_wqkv, A_wo, B_w_gate, B_w_up, B_w_down)
    return out.reshape(1, S, D)
```

```python
import functools
import math

import jax
import jax.numpy as jnp
from jax import lax
from jax.experimental import pallas as pl
from jax.experimental.pallas import tpu as pltpu

S, D, F = 2048, 1024, 3584
H, DH, WIN, DIL = 32, 32, 8, 2
EPS = 1e-5
NEG = -1e9
bf16, f32, u32 = jnp.bfloat16, jnp.float32, jnp.uint32

SB = 256
SBA = 512
FC = 512
R = 8
HALO = 16
WOP = 65
BFLY = ((1, 2), (2, 4), (4, 8))

NS, NQ, NF = S // SB, S // SBA, F // FC
DP, DHALF, KP, FH = D // 2, D // 2, D // 4, FC // 2
HB = SB // 2
XP = HB // 2
NSLAB = 4
SLAB = KP // NSLAB
KSLAB = KP // NS
GR = KP // NQ
DC = DHALF // NQ
A0_DOTS, A1_DOTS, B_FRAC = 6, 6, 0.85
assert NQ == NSLAB and DC % 128 == 0 and GR % 8 == 0 and KSLAB % 8 == 0 and FH % 128 == 0 and (FH // 2) % 8 == 0


def _roll(x, s):
    return pltpu.roll(x, s % 128, 1)


def _lanebit_clear(shape, bit):
    return (lax.broadcasted_iota(jnp.int32, shape, 1) & bit) == 0


def _bfly_stage(t, tb, lb):
    msk = _lanebit_clear(t[0].shape, lb)
    n = [None] * 8
    for a in range(8):
        if a & tb:
            continue
        b = a | tb
        n[a] = jnp.where(msk, t[a], _roll(t[b], lb))
        n[b] = jnp.where(msk, _roll(t[a], -lb), t[b])
    return n


def _silu(x):
    return x * pl.reciprocal(1.0 + jnp.exp(-x), approx=True)


def _dot(a, b):
    return jnp.dot(a, b, preferred_element_type=f32)


def _unpack(t, i):
    return pltpu.unpack_elementwise(t, index=i, packed_dtype=bf16, unpacked_dtype=f32)


def _pack(lo, hi):
    return pltpu.bitcast(pltpu.pack_elementwise([lo, hi], packed_dtype=bf16), u32)


def _w32(ref):
    return ref.bitcast(u32)


def _a_combos(a):
    m, k = a.shape[0] // 2, a.shape[1] // 2
    a11, a12, a21, a22 = a[:m, :k], a[:m, k:], a[m:, :k], a[m:, k:]
    return [t.astype(bf16) for t in (a11 + a22, a21 + a22, a11, a22, a11 + a12, a21 - a11, a12 - a22)]


def _b_combos(b11, b12, b21, b22):
    def five(x11, x12, x21, x22):
        return (x11 + x22, x12 - x22, x21 - x11, x11 + x12, x21 + x22)

    lo = five(*[_unpack(t, 0) for t in (b11, b12, b21, b22)])
    hi = five(*[_unpack(t, 1) for t in (b11, b12, b21, b22)])
    return [_pack(l, h) for l, h in zip(lo, hi)]


def _rhs7(b11, b22, cmb):
    return [pltpu.bitcast(t, bf16) for t in (cmb(0), b11, cmb(1), cmb(2), b22, cmb(3), cmb(4))]


def _c_combos(m):
    return (m[0] + m[3] - m[4] + m[6], m[2] + m[4], m[1] + m[3], m[0] - m[1] + m[2] + m[5])


def _c_full(m):
    c11, c12, c21, c22 = _c_combos(m)
    return jnp.concatenate([jnp.concatenate([c11, c12], axis=1), jnp.concatenate([c21, c22], axis=1)], axis=0)


def _mult(v, m):
    return v if isinstance(v, int) else pl.multiple_of(v, m)


def _kernel(x_hbm, wqkv_hbm, wo_hbm, wg_hbm, wu_hbm, wd_hbm, out_hbm,
            x_v, xl_v, out_v, wq_v, qc_v, wk_v, kc_v, wv_v, vc_v, wo_v, wop, woc,
            wg_v, wu_v, wd_v, gc, uc, dc, q_s, k_s, v_s, o_s, ol_s, z_ref, sems):
    SEM_OUT, SEM_O = 0, 1
    SEM_X = 2
    SEM_Q = SEM_X + NS
    SEM_K = SEM_Q + NSLAB
    SEM_V = SEM_K + NS
    SEM_G = SEM_V + NSLAB
    SEM_D = SEM_G + NQ

    def cp_x(i):
        r0 = _mult(i * SB, SB)
        return pltpu.make_async_copy(x_hbm.at[pl.ds(r0, SB)], x_v.at[pl.ds(r0, SB)], sems.at[SEM_X + i])

    def cp_pair(dst, m, p0, nr, sem):
        cps = []
        for kh in range(2):
            p = _mult(kh * KP + p0, nr)
            cps.append(pltpu.make_async_copy(
                _w32(wqkv_hbm).at[pl.ds(p, nr), pl.ds(m * D, D)], dst.at[pl.ds(p, nr), :], sems.at[sem]))
        return cps

    def cp_q(i):
        return cp_pair(wq_v, 0, i * SLAB, SLAB, SEM_Q + i)

    def cp_k(b):
        return cp_pair(wk_v, 1, b * KSLAB, KSLAB, SEM_K + b)

    def cp_v(i):
        return cp_pair(wv_v, 2, i * SLAB, SLAB, SEM_V + i)

    def cp_o():
        return pltpu.make_async_copy(_w32(wo_hbm), wo_v, sems.at[SEM_O])

    def cp_gu(q):
        cps = []
        for src, dst in ((wg_hbm, wg_v), (wu_hbm, wu_v)):
            for kh in range(2):
                r0 = _mult(kh * KP + q * GR, 8)
                cps.append(pltpu.make_async_copy(
                    _w32(src).at[pl.ds(r0, GR), :], dst.at[pl.ds(r0, GR), :], sems.at[SEM_G + q]))
        return cps

    def cp_d(q):
        cps = []
        for nh in range(2):
            c0 = _mult(nh * DHALF + q * DC, 128)
            cps.append(pltpu.make_async_copy(
                _w32(wd_hbm).at[:, pl.ds(c0, DC)], wd_v.at[:, pl.ds(c0, DC)], sems.at[SEM_D + q]))
        return cps

    def cp_out(r0):
        return pltpu.make_async_copy(out_v.at[pl.ds(r0, SB)], out_hbm.at[pl.ds(r0, SB)], sems.at[SEM_OUT])

    def tied(v, tie):
        if tie is None:
            return v
        if v.shape[1] > 128:
            return jnp.concatenate([tied(v[:, 0:128], tie), v[:, 128:]], axis=1)
        if v.shape[0] > 8:
            return jnp.concatenate([tied(v[0:8], tie), v[8:]], axis=0)
        return pltpu.bitcast(pltpu.bitcast(v, u32) | tie, v.dtype)

    class Pacer:
        def __init__(self, stages, ndots):
            self.stages, self.ndots, self.k, self.done = list(stages), ndots, 0, 0

        def after_dot(self, m):
            self.k += 1
            total = len(self.stages)
            target = total if self.k >= self.ndots else (total * self.k) // self.ndots
            n = target - self.done
            if n <= 0:
                return
            nr, nc = m.shape[0] // 8, m.shape[1] // 128
            zero = z_ref[...]
            for i in range(n):
                c, r = divmod((i * nr * nc) // n, nr)
                self.stages[self.done + i](pltpu.bitcast(m[8 * r:8 * r + 8, 128 * c:128 * (c + 1)], u32) & zero)
            self.done = target

        def flush(self):
            for st in self.stages[self.done:]:
                st(None)
            self.done = len(self.stages)

    def prep_stages(raw, cmb, p0, nr):
        p1, p2 = p0, KP + p0
        tie = yield
        t1 = [raw[pl.ds(p1, nr), 128 * j:128 * (j + 1)] for j in range(8)]
        t2 = [raw[pl.ds(p2, nr), 128 * j:128 * (j + 1)] for j in range(8)]
        for tb, lb in BFLY:
            t1[0] = tied(t1[0], tie)
            t2[0] = tied(t2[0], tie)
            t1, t2 = _bfly_stage(t1, tb, lb), _bfly_stage(t2, tb, lb)
            tie = yield
        t1[0] = tied(t1[0], tie)
        for j in range(4):
            raw[pl.ds(p1, nr), 128 * j:128 * (j + 1)] = t1[j]
            raw[pl.ds(p2, nr), 128 * (4 + j):128 * (5 + j)] = t2[4 + j]
            o = _b_combos(t1[j], t1[4 + j], t2[j], t2[4 + j])
            for k in range(5):
                cmb[k, pl.ds(p1, nr), 128 * j:128 * (j + 1)] = o[k]
        yield

    def run_all(gen, nstages):
        next(gen)
        for _ in range(nstages):
            gen.send(None)

    def prep_pair(raw, cmb, p0, nr, tie=None):
        gen = prep_stages(raw, cmb, p0, nr)
        next(gen)
        gen.send(tie)
        for _ in range(3):
            gen.send(None)

    def qkv_rhs(raw, cmb):
        return _rhs7(raw[0:KP, 0:DHALF], raw[KP:2 * KP, DHALF:D], lambda k: cmb[k])

    def gu_pieces(q):
        r0 = pl.multiple_of(q * GR, 8)

        def piece(raw, dst, f, ct, rr, tie=None):
            cl, cr = f * FC + ct * 128, f * FC + FH + ct * 128
            o = _b_combos(tied(raw[pl.ds(r0 + rr, 8), cl:cl + 128], tie), raw[pl.ds(r0 + rr, 8), cr:cr + 128],
                          raw[pl.ds(KP + r0 + rr, 8), cl:cl + 128], raw[pl.ds(KP + r0 + rr, 8), cr:cr + 128])
            for k in range(5):
                dst[k, pl.ds(r0 + rr, 8), f * FH + ct * 128:f * FH + (ct + 1) * 128] = o[k]

        return [functools.partial(piece, raw, dst, f, ct, rr)
                for raw, dst in ((wg_v, gc), (wu_v, uc))
                for f in range(NF) for ct in range(FH // 128) for rr in range(0, GR, 8)]

    def d_pieces(q):
        c0 = pl.multiple_of(q * DC, 128)
        kq = FH // 2

        def piece(f, rr, cc, tie=None):
            k0 = f * FH + rr
            o = _b_combos(tied(wd_v[k0:k0 + 8, pl.ds(c0 + cc, 128)], tie), wd_v[k0:k0 + 8, pl.ds(DHALF + c0 + cc, 128)],
                          wd_v[k0 + kq:k0 + kq + 8, pl.ds(c0 + cc, 128)],
                          wd_v[k0 + kq:k0 + kq + 8, pl.ds(DHALF + c0 + cc, 128)])
            for k in range(5):
                dc[k, f * kq + rr:f * kq + rr + 8, pl.ds(c0 + cc, 128)] = o[k]

        return [functools.partial(piece, f, rr, cc)
                for f in range(NF) for cc in range(0, DC, 128) for rr in range(0, kq, 8)]

    def wo_pieces(q):
        def plane(ct, T, tie=None):
            blk = tied(wo_v[64 * T:64 * (T + 1), pl.ds(pl.multiple_of(ct * 128, 128), 128)], tie)
            for c in range(8):
                wop[ct, pl.ds(8 * c + T, 8, stride=WOP), :] = blk[8 * c:8 * c + 8, :]

        def combo(jj, rr, tie=None):
            r1, r2 = WOP * jj + rr, WOP * (4 + jj) + rr
            o = _b_combos(tied(wop[q, r1:r1 + 8, :], tie), wop[4 + q, r1:r1 + 8, :],
                          wop[q, r2:r2 + 8, :], wop[4 + q, r2:r2 + 8, :])
            for k in range(5):
                woc[k, 64 * jj + rr:64 * jj + rr + 8, pl.ds(pl.multiple_of(q * 128, 128), 128)] = o[k]

        out = [functools.partial(plane, ct, T) for T in range(8) for ct in (q, 4 + q)]
        return out + [functools.partial(combo, jj, rr) for jj in range(4) for rr in range(0, 64, 8)]

    def wo_tile(j0, j1, c0, c1):
        return jnp.concatenate(
            [jnp.concatenate([wop[ct, WOP * j:WOP * j + 64, :] for ct in range(c0, c1)], axis=1) for j in range(j0, j1)],
            axis=0)

    def ln_stages(b, u0, nu):
        r0 = _mult(b * SB, SB) + 16 * u0
        tie = yield
        x = jnp.concatenate([tied(x_v[pl.ds(r0, 16 * nu), :].astype(f32), tie),
                             x_v[pl.ds(r0 + HB, 16 * nu), :].astype(f32)], axis=0)
        mean = jnp.mean(x, axis=-1, keepdims=True)
        tie = yield
        xc = tied(x - mean, tie)
        var = jnp.mean(xc * xc, axis=-1, keepdims=True)
        tie = yield
        xn = tied(xc, tie) * lax.rsqrt(var + EPS)
        p0 = _mult(b * XP, XP) + 8 * u0
        for k, l in enumerate(_a_combos(xn)):
            xl_v[k, pl.ds(p0, 8 * nu), :] = pltpu.bitcast(l, u32)
        yield

    def xl_lhs(p0, n):
        return [pltpu.bitcast(xl_v[k, pl.ds(p0, n), :], bf16) for k in range(7)]

    def store_planes(dst, row0, nblk, m):
        c11, c12, c21, c22 = _c_combos(m)
        for blk in range(nblk):
            for half, (cl, cr) in enumerate(((c11, c12), (c21, c22))):
                r = row0 + blk * SB + half * HB
                for j in range(4):
                    dst[j, pl.ds(r, HB), :] = cl[blk * HB:(blk + 1) * HB, 128 * j:128 * (j + 1)]
                    dst[4 + j, pl.ds(r, HB), :] = cr[blk * HB:(blk + 1) * HB, 128 * j:128 * (j + 1)]

    def paced_product(lhs, rhs, stages, ndots):
        pacer = Pacer(stages, ndots)
        m = []
        for l, w in zip(lhs, rhs):
            m.append(_dot(l, w))
            pacer.after_dot(m[-1])
        pacer.flush()
        return m

    def body_a0(b, carry):
        @pl.when(b < NS - 1)
        def _():
            cp_x(b + 1).wait()
        for cp in cp_k(b):
            cp.wait()
        lhs = xl_lhs(pl.multiple_of(b * XP, XP), XP)
        nxt = jnp.minimum(b + 1, NS - 1)
        p0 = pl.multiple_of(b * KSLAB, KSLAB)
        gens = []
        for u in range(HB // 16):
            gens.append((ln_stages(nxt, u, 1), 3))
            if u % 2 == 0:
                gens.append((prep_stages(wk_v, kc_v, p0 + 4 * u, 8), 4))
        for g, _ in gens:
            next(g)
        stages = [g.send for st in range(4) for g, n in gens if st < n]
        m = paced_product(lhs, qkv_rhs(wq_v, qc_v), stages, A0_DOTS)
        store_planes(q_s, pl.multiple_of(b * SB, SB), 1, m)
        return carry

    def kv_proj(b, raw, cmb, dst, stages):
        nblk = SBA // SB
        lhs = xl_lhs(pl.multiple_of(b * nblk * XP, XP), nblk * XP)
        m = paced_product(lhs, qkv_rhs(raw, cmb), stages, A1_DOTS)
        store_planes(dst, pl.multiple_of(b * SBA, SBA) + HALO, nblk, m)

    def body_ak(b, carry):
        for cp in cp_v(b) + cp_gu(b):
            cp.wait()
        p0 = pl.multiple_of(b * SLAB, SLAB)
        vst = [functools.partial(prep_pair, wv_v, vc_v, p0 + 8 * u, 8) for u in range(SLAB // 8)]
        gu = gu_pieces(b)
        every = len(gu) // len(vst)
        stages = []
        for i, st in enumerate(gu):
            if i % every == 0:
                stages.append(vst[i // every])
            stages.append(st)
        kv_proj(b, wk_v, kc_v, k_s, stages)
        return carry

    def body_av(b, carry):
        @pl.when(b == 0)
        def _():
            cp_o().wait()
        for cp in cp_d(b):
            cp.wait()
        kv_proj(b, wv_v, vc_v, v_s, wo_pieces(b) + d_pieces(b))
        return carry

    shp = (R, 128)
    SCALE = DH ** -0.5
    CEXP = SCALE * math.log2(math.e)

    def body_b(b, carry):
        r_off = pl.multiple_of(b * SB, SB)
        m16 = _lanebit_clear(shp, 16)
        m1 = _lanebit_clear(shp, 1)
        xl = xl_lhs(pl.multiple_of(b * XP, XP), XP)

        def swap(z, msk, s):
            return jnp.where(msk, _roll(z, -s), _roll(z, s))

        def merge(p, q, msk, s):
            return jnp.where(msk, p + _roll(p, -s), q + _roll(q, s))

        def tree_sum(ts):
            while len(ts) > 1:
                ts = [ts[i] + ts[i + 1] for i in range(0, len(ts), 2)]
            return ts[0]

        def attn_rows(r0):
            q = None
            P = []
            for w in range(WIN):
                tie = yield
                if q is None:
                    q = [q_s[j, pl.ds(r_off + r0, R), :] for j in range(8)]
                base = r_off + (HALO + r0 - DIL * w)
                kk = [k_s[j, pl.ds(base, R), :] for j in range(8)]
                kk[0] = tied(kk[0], tie)
                P.append(tree_sum([q[j] * kk[j] for j in range(8)]))
            z0 = merge(merge(P[0], P[1], m16, 16), merge(P[2], P[3], m16, 16), m1, 1)
            z1 = merge(merge(P[4], P[5], m16, 16), merge(P[6], P[7], m16, 16), m1, 1)
            if r0 < DIL * (WIN - 1):
                lane = lax.broadcasted_iota(jnp.int32, shp, 1)
                row = lax.broadcasted_iota(jnp.int32, shp, 0) + (r0 + r_off)
                w0 = ((lane >> 4) & 1) + 2 * (lane & 1)
                z0 = jnp.where(row >= DIL * w0, z0, NEG / SCALE)
                z1 = jnp.where(row >= DIL * (w0 + 4), z1, NEG / SCALE)
            mx = jnp.maximum(z0, z1)
            mx = jnp.maximum(mx, swap(mx, m16, 16))
            mx = jnp.maximum(mx, swap(mx, m1, 1))
            e0 = jnp.exp2((z0 - mx) * CEXP)
            e1 = jnp.exp2((z1 - mx) * CEXP)
            den = e0 + e1
            den = den + swap(den, m16, 16)
            den = den + swap(den, m1, 1)
            inv = 1.0 / den
            a = []
            for e in (e0 * inv, e1 * inv):
                u0 = jnp.where(m1, e, _roll(e, 1))
                u1 = jnp.where(m1, _roll(e, -1), e)
                for u in (u0, u1):
                    a.append(jnp.where(m16, u, _roll(u, 16)))
                    a.append(jnp.where(m16, _roll(u, -16), u))
            for j in range(8):
                tie = yield
                vv = [v_s[j, pl.ds(r_off + (HALO + r0 - DIL * w), R), :] for w in range(WIN)]
                vv[0] = tied(vv[0], tie)
                o_s[r0:r0 + R, 128 * j:128 * (j + 1)] = tree_sum([a[w] * vv[w] for w in range(WIN)])
            yield

        def o_combos(u, tie):
            top = tied(o_s[16 * u:16 * u + 16, :], tie)
            o = jnp.concatenate([top, o_s[HB + 16 * u:HB + 16 * u + 16, :]], axis=0)
            for k, l in enumerate(_a_combos(o)):
                ol_s[k, 8 * u:8 * u + 8, :] = pltpu.bitcast(l, u32)

        stages = []
        for u in range(HB // 16):
            for g0 in (16 * u, HB + 16 * u):
                for r0 in range(g0, g0 + 16, R):
                    gen = attn_rows(r0)
                    next(gen)
                    stages += [gen.send] * (2 * WIN)
            stages.append(functools.partial(o_combos, u))
        pacer = Pacer(stages, int((21 * NF - 7) * B_FRAC))

        def pdots(lhs, rhs):
            m = []
            for l, w in zip(lhs, rhs):
                m.append(_dot(l, w))
                pacer.after_dot(m[-1])
            return m

        def gu_rhs(raw, cmb, f):
            return _rhs7(raw[0:KP, f * FC:f * FC + FH], raw[KP:2 * KP, f * FC + FH:(f + 1) * FC],
                         lambda k: cmb[k, :, f * FH:(f + 1) * FH])

        def d_rhs(f):
            k0, kq = f * FH, FH // 2
            return _rhs7(wd_v[k0:k0 + kq, 0:DHALF], wd_v[k0 + kq:k0 + 2 * kq, DHALF:D],
                         lambda k: dc[k, f * kq:(f + 1) * kq, :])

        acc, pend = None, None
        for f in range(NF):
            gt = _c_full(pdots(xl, gu_rhs(wg_v, gc, f)))
            up = _c_full(pdots(xl, gu_rhs(wu_v, uc, f)))
            hl = _a_combos(_silu(gt) * up)
            if pend is not None:
                d = pdots(pend[1], d_rhs(pend[0]))
                acc = d if acc is None else [p + t for p, t in zip(acc, d)]
            pend = (f, hl)
        acc = [p + t for p, t in zip(acc, pdots(pend[1], d_rhs(pend[0])))]
        y = _c_full(acc)
        pacer.flush()
        rhs = _rhs7(wo_tile(0, 4, 0, 4), wo_tile(4, 8, 4, 8), lambda k: woc[k])
        s = _c_full([_dot(pltpu.bitcast(ol_s[k], bf16), rhs[k]) for k in range(7)])
        xr = x_v[pl.ds(r_off, SB), :].astype(f32)
        out_v[pl.ds(r_off, SB), :] = (xr + s * _silu(y)).astype(out_v.dtype)
        cp_out(r_off).start()
        return carry

    cp_x(0).start()
    for i in range(NSLAB):
        for cp in cp_q(i):
            cp.start()
    for b in range(NS):
        if b + 1 < NS:
            cp_x(b + 1).start()
        for cp in cp_k(b):
            cp.start()
    for q in range(NQ):
        for cp in cp_v(q) + cp_gu(q):
            cp.start()
    cp_o().start()
    for q in range(NQ):
        for cp in cp_d(q):
            cp.start()
    z_ref[...] = jnp.zeros((8, 128), u32)
    k_s[:, 0:HALO, :] = jnp.zeros((8, HALO, 128), f32)
    v_s[:, 0:HALO, :] = jnp.zeros((8, HALO, 128), f32)
    cp_x(0).wait()
    run_all(ln_stages(0, 0, HB // 16), 3)

    def body_prep(i, carry):
        for cp in cp_q(i):
            cp.wait()
        prep_pair(wq_v, qc_v, pl.multiple_of(i * SLAB, SLAB), SLAB)
        return carry

    lax.fori_loop(0, NSLAB, body_prep, 0)
    lax.fori_loop(0, NS, body_a0, 0)
    lax.fori_loop(0, NQ, body_ak, 0)
    lax.fori_loop(0, NQ, body_av, 0)
    lax.fori_loop(0, NS, body_b, 0)
    for i in range(NS):
        cp_out(i * SB).wait()


def _scratch_shapes():
    vm = pltpu.VMEM
    return [
        vm((S, D), bf16), vm((7, S // 4, DHALF), u32), vm((S, D), bf16),
        vm((DP, D), u32), vm((5, KP, DHALF), u32),
        vm((DP, D), u32), vm((5, KP, DHALF), u32),
        vm((DP, D), u32), vm((5, KP, DHALF), u32),
        vm((DP, D), u32), vm((8, 8 * WOP, 128), u32), vm((5, KP, DHALF), u32),
        vm((DP, F), u32), vm((DP, F), u32), vm((F // 2, D), u32),
        vm((5, KP, F // 2), u32), vm((5, KP, F // 2), u32), vm((5, F // 4, DHALF), u32),
        vm((8, S, 128), f32), vm((8, HALO + S, 128), f32), vm((8, HALO + S, 128), f32),
        vm((SB, D), f32), vm((7, XP, DHALF), u32), vm((8, 128), u32),
        pltpu.SemaphoreType.DMA((2 + 2 * NS + 2 * NSLAB + 2 * NQ,)),
    ]


@jax.jit
def pallas_recurrent_scan__sliding_local_dilated__swiglu_ffn__prompt_kernel(
    A_x: jax.Array,
    A_wqkv: jax.Array,
    A_wo: jax.Array,
    B_x: jax.Array,
    B_w_gate: jax.Array,
    B_w_up: jax.Array,
    B_w_down: jax.Array,
):
    del B_x
    assert A_x.shape == (1, S, D) and A_wqkv.shape == (D, 3 * D) and B_w_gate.shape == (D, F)
    any_spec = pl.BlockSpec(memory_space=pl.ANY)
    out = pl.pallas_call(
        _kernel,
        in_specs=[any_spec] * 6,
        out_specs=any_spec,
        out_shape=jax.ShapeDtypeStruct((S, D), bf16),
        scratch_shapes=_scratch_shapes(),
        compiler_params=pltpu.CompilerParams(vmem_limit_bytes=124 << 20),
        name="fused_attn_swiglu",
    )(A_x.reshape(S, D), A_wqkv, A_wo, B_w_gate, B_w_up, B_w_down)
    return out.reshape(1, S, D)
```

```python
import functools
import math

import jax
import jax.numpy as jnp
from jax import lax
from jax.experimental import pallas as pl
from jax.experimental.pallas import tpu as pltpu

S, D, F = 2048, 1024, 3584
H, DH, WIN, DIL = 32, 32, 8, 2
EPS = 1e-5
NEG = -1e9
bf16, f32, u32 = jnp.bfloat16, jnp.float32, jnp.uint32

SB = 256
SBA = 512
FC = 512
R = 8
HALO = 16
WOP = 65
BFLY = ((1, 2), (2, 4), (4, 8))

NS, NQ, NF = S // SB, S // SBA, F // FC
DHALF, KP, FH = D // 2, D // 4, FC // 2
HB = SB // 2
XP = HB // 2
NSLAB = 4
SLAB = KP // NSLAB
KSLAB = KP // NS
GR = KP // NQ
DC = DHALF // NQ
A0_DOTS, A1_DOTS, B_FRAC = 6, 6, 0.85
assert NQ == NSLAB and DC % 128 == 0 and GR % 8 == 0 and KSLAB % 8 == 0 and FH % 128 == 0 and (FH // 2) % 8 == 0


def _roll(x, s):
    return pltpu.roll(x, s % 128, 1)


def _lanebit_clear(shape, bit):
    return (lax.broadcasted_iota(jnp.int32, shape, 1) & bit) == 0


def _bfly_stage(t, tb, lb):
    msk = _lanebit_clear(t[0].shape, lb)
    n = [None] * 8
    for a in range(8):
        if a & tb:
            continue
        b = a | tb
        n[a] = jnp.where(msk, t[a], _roll(t[b], lb))
        n[b] = jnp.where(msk, _roll(t[a], -lb), t[b])
    return n


def _silu(x):
    return x * pl.reciprocal(1.0 + jnp.exp(-x), approx=True)


def _dot(a, b):
    return jnp.dot(a, b, preferred_element_type=f32)


def _a_combos(a):
    m, k = a.shape[0] // 2, a.shape[1] // 2
    a11, a12, a21, a22 = a[:m, :k], a[:m, k:], a[m:, :k], a[m:, k:]
    return [t.astype(bf16) for t in (a11 + a22, a21 + a22, a11, a22, a11 + a12, a21 - a11, a12 - a22)]


def _b_combos(b11, b12, b21, b22):
    x11, x12, x21, x22 = [t.astype(f32) for t in (b11, b12, b21, b22)]
    return [pltpu.bitcast(t.astype(bf16), u32) for t in (x11 + x22, x12 - x22, x21 - x11, x11 + x12, x21 + x22)]


def _rhs7(b11, b22, cmb):
    c = [pltpu.bitcast(cmb(k), bf16) for k in range(5)]
    return [c[0], b11, c[1], c[2], b22, c[3], c[4]]


def _c_combos(m):
    return (m[0] + m[3] - m[4] + m[6], m[2] + m[4], m[1] + m[3], m[0] - m[1] + m[2] + m[5])


def _c_full(m):
    c11, c12, c21, c22 = _c_combos(m)
    return jnp.concatenate([jnp.concatenate([c11, c12], axis=1), jnp.concatenate([c21, c22], axis=1)], axis=0)


def _mult(v, m):
    return v if isinstance(v, int) else pl.multiple_of(v, m)


def _kernel(x_hbm, wqkv_hbm, wo_hbm, wg_hbm, wu_hbm, wd_hbm, out_hbm,
            x_v, xl_v, out_v, wq_v, qc_v, wk_v, kc_v, wv_v, vc_v, wo_v, wop, woc,
            wg_v, wu_v, wd_v, gc, uc, dc, q_s, k_s, v_s, o_s, ol_s, z_ref, sems):
    SEM_OUT, SEM_O = 0, 1
    SEM_X = 2
    SEM_Q = SEM_X + NS
    SEM_K = SEM_Q + NSLAB
    SEM_V = SEM_K + NS
    SEM_G = SEM_V + NSLAB
    SEM_D = SEM_G + NQ

    def cp_x(i):
        r0 = _mult(i * SB, SB)
        return pltpu.make_async_copy(x_hbm.at[pl.ds(r0, SB)], x_v.at[pl.ds(r0, SB)], sems.at[SEM_X + i])

    def cp_pair(dst, m, p0, nr, sem):
        cps = []
        for kh in range(2):
            r = _mult(2 * (kh * KP + p0), 2 * nr)
            cps.append(pltpu.make_async_copy(
                wqkv_hbm.at[pl.ds(r, 2 * nr), pl.ds(m * D, D)], dst.at[pl.ds(r, 2 * nr), :], sems.at[sem]))
        return cps

    def cp_q(i):
        return cp_pair(wq_v, 0, i * SLAB, SLAB, SEM_Q + i)

    def cp_k(b):
        return cp_pair(wk_v, 1, b * KSLAB, KSLAB, SEM_K + b)

    def cp_v(i):
        return cp_pair(wv_v, 2, i * SLAB, SLAB, SEM_V + i)

    def cp_o():
        return pltpu.make_async_copy(wo_hbm, wo_v, sems.at[SEM_O])

    def cp_gu(q):
        cps = []
        for src, dst in ((wg_hbm, wg_v), (wu_hbm, wu_v)):
            for kh in range(2):
                r0 = _mult(2 * (kh * KP + q * GR), 16)
                cps.append(pltpu.make_async_copy(
                    src.at[pl.ds(r0, 2 * GR), :], dst.at[pl.ds(r0, 2 * GR), :], sems.at[SEM_G + q]))
        return cps

    def cp_d(q):
        cps = []
        for nh in range(2):
            c0 = _mult(nh * DHALF + q * DC, 128)
            cps.append(pltpu.make_async_copy(
                wd_hbm.at[:, pl.ds(c0, DC)], wd_v.at[:, pl.ds(c0, DC)], sems.at[SEM_D + q]))
        return cps

    def cp_out(r0):
        return pltpu.make_async_copy(out_v.at[pl.ds(r0, SB)], out_hbm.at[pl.ds(r0, SB)], sems.at[SEM_OUT])

    def tied(v, tie):
        if tie is None:
            return v
        if v.shape[1] > 128:
            return jnp.concatenate([tied(v[:, 0:128], tie), v[:, 128:]], axis=1)
        if v.shape[0] > 8:
            return jnp.concatenate([tied(v[0:8], tie), v[8:]], axis=0)
        return pltpu.bitcast(pltpu.bitcast(v, u32) | tie, v.dtype)

    class Pacer:
        def __init__(self, stages, ndots):
            self.stages, self.ndots, self.k, self.done = list(stages), ndots, 0, 0

        def after_dot(self, m):
            self.k += 1
            total = len(self.stages)
            target = total if self.k >= self.ndots else (total * self.k) // self.ndots
            n = target - self.done
            if n <= 0:
                return
            nr, nc = m.shape[0] // 8, m.shape[1] // 128
            zero = z_ref[...]
            for i in range(n):
                c, r = divmod((i * nr * nc) // n, nr)
                self.stages[self.done + i](pltpu.bitcast(m[8 * r:8 * r + 8, 128 * c:128 * (c + 1)], u32) & zero)
            self.done = target

        def flush(self):
            for st in self.stages[self.done:]:
                st(None)
            self.done = len(self.stages)

    def prep_stages(raw, cmb, p0, nr):
        p1, p2 = 2 * p0, 2 * (KP + p0)
        tie = yield
        t1 = [pltpu.bitcast(raw[pl.ds(p1, 2 * nr), 128 * j:128 * (j + 1)], u32) for j in range(8)]
        t2 = [pltpu.bitcast(raw[pl.ds(p2, 2 * nr), 128 * j:128 * (j + 1)], u32) for j in range(8)]
        for tb, lb in BFLY:
            t1[0] = tied(t1[0], tie)
            t2[0] = tied(t2[0], tie)
            t1, t2 = _bfly_stage(t1, tb, lb), _bfly_stage(t2, tb, lb)
            tie = yield
        t1[0] = tied(t1[0], tie)
        t1, t2 = [pltpu.bitcast(t, bf16) for t in t1], [pltpu.bitcast(t, bf16) for t in t2]
        for j in range(4):
            raw[pl.ds(p1, 2 * nr), 128 * j:128 * (j + 1)] = t1[j]
            raw[pl.ds(p2, 2 * nr), 128 * (4 + j):128 * (5 + j)] = t2[4 + j]
            o = _b_combos(t1[j], t1[4 + j], t2[j], t2[4 + j])
            for k in range(5):
                cmb[k, pl.ds(p0, nr), 128 * j:128 * (j + 1)] = o[k]
        yield

    def run_all(gen, nstages):
        next(gen)
        for _ in range(nstages):
            gen.send(None)

    def prep_pair(raw, cmb, p0, nr, tie=None):
        gen = prep_stages(raw, cmb, p0, nr)
        next(gen)
        gen.send(tie)
        for _ in range(3):
            gen.send(None)

    def qkv_rhs(raw, cmb):
        return _rhs7(raw[0:DHALF, 0:DHALF], raw[DHALF:D, DHALF:D], lambda k: cmb[k])

    def gu_pieces(q):
        r0 = pl.multiple_of(q * 2 * GR, 16)
        rp = pl.multiple_of(q * GR, 8)

        def piece(raw, dst, f, ct, rr, tie=None):
            cl, cr = f * FC + ct * 128, f * FC + FH + ct * 128
            o = _b_combos(tied(raw[pl.ds(r0 + rr, 16), cl:cl + 128].astype(f32), tie), raw[pl.ds(r0 + rr, 16), cr:cr + 128],
                          raw[pl.ds(DHALF + r0 + rr, 16), cl:cl + 128], raw[pl.ds(DHALF + r0 + rr, 16), cr:cr + 128])
            for k in range(5):
                dst[k, pl.ds(rp + rr // 2, 8), f * FH + ct * 128:f * FH + (ct + 1) * 128] = o[k]

        return [functools.partial(piece, raw, dst, f, ct, rr)
                for raw, dst in ((wg_v, gc), (wu_v, uc))
                for f in range(NF) for ct in range(FH // 128) for rr in range(0, 2 * GR, 16)]

    def d_pieces(q):
        c0 = pl.multiple_of(q * DC, 128)

        def piece(f, rr, cc, tie=None):
            k0 = f * FC + rr
            o = _b_combos(tied(wd_v[k0:k0 + 16, pl.ds(c0 + cc, 128)].astype(f32), tie),
                          wd_v[k0:k0 + 16, pl.ds(DHALF + c0 + cc, 128)],
                          wd_v[k0 + FH:k0 + FH + 16, pl.ds(c0 + cc, 128)],
                          wd_v[k0 + FH:k0 + FH + 16, pl.ds(DHALF + c0 + cc, 128)])
            for k in range(5):
                dc[k, (f * FH + rr) // 2:(f * FH + rr) // 2 + 8, pl.ds(c0 + cc, 128)] = o[k]

        return [functools.partial(piece, f, rr, cc)
                for f in range(NF) for cc in range(0, DC, 128) for rr in range(0, FH, 16)]

    def wo_pieces(q):
        def plane(ct, T, tie=None):
            blk = tied(pltpu.bitcast(wo_v[128 * T:128 * (T + 1), pl.ds(pl.multiple_of(ct * 128, 128), 128)], u32), tie)
            for c in range(8):
                wop[ct, pl.ds(8 * c + T, 8, stride=WOP), :] = blk[8 * c:8 * c + 8, :]

        def combo(jj, rr, tie=None):
            r1, r2 = WOP * jj + rr, WOP * (4 + jj) + rr
            o = _b_combos(*[pltpu.bitcast(t, bf16) for t in (tied(wop[q, r1:r1 + 8, :], tie), wop[4 + q, r1:r1 + 8, :],
                                                             wop[q, r2:r2 + 8, :], wop[4 + q, r2:r2 + 8, :])])
            for k in range(5):
                woc[k, 64 * jj + rr:64 * jj + rr + 8, pl.ds(pl.multiple_of(q * 128, 128), 128)] = o[k]

        out = [functools.partial(plane, ct, T) for T in range(8) for ct in (q, 4 + q)]
        return out + [functools.partial(combo, jj, rr) for jj in range(4) for rr in range(0, 64, 8)]

    def wo_tile(j0, j1, c0, c1):
        return pltpu.bitcast(jnp.concatenate(
            [jnp.concatenate([wop[ct, WOP * j:WOP * j + 64, :] for ct in range(c0, c1)], axis=1) for j in range(j0, j1)],
            axis=0), bf16)

    def ln_stages(b, u0, nu):
        r0 = _mult(b * SB, SB) + 16 * u0
        tie = yield
        x = jnp.concatenate([tied(x_v[pl.ds(r0, 16 * nu), :].astype(f32), tie),
                             x_v[pl.ds(r0 + HB, 16 * nu), :].astype(f32)], axis=0)
        mean = jnp.mean(x, axis=-1, keepdims=True)
        tie = yield
        xc = tied(x - mean, tie)
        var = jnp.mean(xc * xc, axis=-1, keepdims=True)
        tie = yield
        xn = tied(xc, tie) * lax.rsqrt(var + EPS)
        p0 = _mult(b * XP, XP) + 8 * u0
        for k, l in enumerate(_a_combos(xn)):
            xl_v[k, pl.ds(p0, 8 * nu), :] = pltpu.bitcast(l, u32)
        yield

    def xl_lhs(p0, n):
        return [pltpu.bitcast(xl_v[k, pl.ds(p0, n), :], bf16) for k in range(7)]

    def store_planes(dst, row0, nblk, m):
        c11, c12, c21, c22 = _c_combos(m)
        for blk in range(nblk):
            for half, (cl, cr) in enumerate(((c11, c12), (c21, c22))):
                r = row0 + blk * SB + half * HB
                for j in range(4):
                    dst[j, pl.ds(r, HB), :] = cl[blk * HB:(blk + 1) * HB, 128 * j:128 * (j + 1)]
                    dst[4 + j, pl.ds(r, HB), :] = cr[blk * HB:(blk + 1) * HB, 128 * j:128 * (j + 1)]

    def paced_product(lhs, rhs, stages, ndots):
        pacer = Pacer(stages, ndots)
        m = []
        for l, w in zip(lhs, rhs):
            m.append(_dot(l, w))
            pacer.after_dot(m[-1])
        pacer.flush()
        return m

    def body_a0(b, carry):
        @pl.when(b < NS - 1)
        def _():
            cp_x(b + 1).wait()
        for cp in cp_k(b):
            cp.wait()
        lhs = xl_lhs(pl.multiple_of(b * XP, XP), XP)
        nxt = jnp.minimum(b + 1, NS - 1)
        p0 = pl.multiple_of(b * KSLAB, KSLAB)
        gens = []
        for u in range(HB // 16):
            gens.append((ln_stages(nxt, u, 1), 3))
            if u % 2 == 0:
                gens.append((prep_stages(wk_v, kc_v, p0 + 4 * u, 8), 4))
        for g, _ in gens:
            next(g)
        stages = [g.send for st in range(4) for g, n in gens if st < n]
        m = paced_product(lhs, qkv_rhs(wq_v, qc_v), stages, A0_DOTS)
        store_planes(q_s, pl.multiple_of(b * SB, SB), 1, m)
        return carry

    def kv_proj(b, raw, cmb, dst, stages):
        nblk = SBA // SB
        lhs = xl_lhs(pl.multiple_of(b * nblk * XP, XP), nblk * XP)
        m = paced_product(lhs, qkv_rhs(raw, cmb), stages, A1_DOTS)
        store_planes(dst, pl.multiple_of(b * SBA, SBA) + HALO, nblk, m)

    def body_ak(b, carry):
        for cp in cp_v(b) + cp_gu(b):
            cp.wait()
        p0 = pl.multiple_of(b * SLAB, SLAB)
        vst = [functools.partial(prep_pair, wv_v, vc_v, p0 + 8 * u, 8) for u in range(SLAB // 8)]
        gu = gu_pieces(b)
        every = len(gu) // len(vst)
        stages = []
        for i, st in enumerate(gu):
            if i % every == 0:
                stages.append(vst[i // every])
            stages.append(st)
        kv_proj(b, wk_v, kc_v, k_s, stages)
        return carry

    def body_av(b, carry):
        @pl.when(b == 0)
        def _():
            cp_o().wait()
        for cp in cp_d(b):
            cp.wait()
        kv_proj(b, wv_v, vc_v, v_s, wo_pieces(b) + d_pieces(b))
        return carry

    shp = (R, 128)
    SCALE = DH ** -0.5
    CEXP = SCALE * math.log2(math.e)

    def body_b(b, carry):
        r_off = pl.multiple_of(b * SB, SB)
        m16 = _lanebit_clear(shp, 16)
        m1 = _lanebit_clear(shp, 1)
        xl = xl_lhs(pl.multiple_of(b * XP, XP), XP)

        def swap(z, msk, s):
            return jnp.where(msk, _roll(z, -s), _roll(z, s))

        def merge(p, q, msk, s):
            return jnp.where(msk, p + _roll(p, -s), q + _roll(q, s))

        def tree_sum(ts):
            while len(ts) > 1:
                ts = [ts[i] + ts[i + 1] for i in range(0, len(ts), 2)]
            return ts[0]

        def attn_rows(r0):
            q = None
            P = []
            for w in range(WIN):
                tie = yield
                if q is None:
                    q = [q_s[j, pl.ds(r_off + r0, R), :] for j in range(8)]
                base = r_off + (HALO + r0 - DIL * w)
                kk = [k_s[j, pl.ds(base, R), :] for j in range(8)]
                kk[0] = tied(kk[0], tie)
                P.append(tree_sum([q[j] * kk[j] for j in range(8)]))
            z0 = merge(merge(P[0], P[1], m16, 16), merge(P[2], P[3], m16, 16), m1, 1)
            z1 = merge(merge(P[4], P[5], m16, 16), merge(P[6], P[7], m16, 16), m1, 1)
            if r0 < DIL * (WIN - 1):
                lane = lax.broadcasted_iota(jnp.int32, shp, 1)
                row = lax.broadcasted_iota(jnp.int32, shp, 0) + (r0 + r_off)
                w0 = ((lane >> 4) & 1) + 2 * (lane & 1)
                z0 = jnp.where(row >= DIL * w0, z0, NEG / SCALE)
                z1 = jnp.where(row >= DIL * (w0 + 4), z1, NEG / SCALE)
            mx = jnp.maximum(z0, z1)
            mx = jnp.maximum(mx, swap(mx, m16, 16))
            mx = jnp.maximum(mx, swap(mx, m1, 1))
            e0 = jnp.exp2((z0 - mx) * CEXP)
            e1 = jnp.exp2((z1 - mx) * CEXP)
            den = e0 + e1
            den = den + swap(den, m16, 16)
            den = den + swap(den, m1, 1)
            inv = 1.0 / den
            a = []
            for e in (e0 * inv, e1 * inv):
                u0 = jnp.where(m1, e, _roll(e, 1))
                u1 = jnp.where(m1, _roll(e, -1), e)
                for u in (u0, u1):
                    a.append(jnp.where(m16, u, _roll(u, 16)))
                    a.append(jnp.where(m16, _roll(u, -16), u))
            for j in range(8):
                tie = yield
                vv = [v_s[j, pl.ds(r_off + (HALO + r0 - DIL * w), R), :] for w in range(WIN)]
                vv[0] = tied(vv[0], tie)
                o_s[r0:r0 + R, 128 * j:128 * (j + 1)] = tree_sum([a[w] * vv[w] for w in range(WIN)])
            yield

        def o_combos(u, tie):
            top = tied(o_s[16 * u:16 * u + 16, :], tie)
            o = jnp.concatenate([top, o_s[HB + 16 * u:HB + 16 * u + 16, :]], axis=0)
            for k, l in enumerate(_a_combos(o)):
                ol_s[k, 8 * u:8 * u + 8, :] = pltpu.bitcast(l, u32)

        stages = []
        for u in range(HB // 16):
            for g0 in (16 * u, HB + 16 * u):
                for r0 in range(g0, g0 + 16, R):
                    gen = attn_rows(r0)
                    next(gen)
                    stages += [gen.send] * (2 * WIN)
            stages.append(functools.partial(o_combos, u))
        pacer = Pacer(stages, int((21 * NF - 7) * B_FRAC))

        def pdots(lhs, rhs):
            m = []
            for l, w in zip(lhs, rhs):
                m.append(_dot(l, w))
                pacer.after_dot(m[-1])
            return m

        def gu_rhs(raw, cmb, f):
            return _rhs7(raw[0:DHALF, f * FC:f * FC + FH], raw[DHALF:D, f * FC + FH:(f + 1) * FC],
                         lambda k: cmb[k, :, f * FH:(f + 1) * FH])

        def d_rhs(f):
            k0 = f * FC
            return _rhs7(wd_v[k0:k0 + FH, 0:DHALF], wd_v[k0 + FH:k0 + FC, DHALF:D],
                         lambda k: dc[k, f * FH // 2:(f + 1) * FH // 2, :])

        acc, pend = None, None
        for f in range(NF):
            gt = _c_full(pdots(xl, gu_rhs(wg_v, gc, f)))
            up = _c_full(pdots(xl, gu_rhs(wu_v, uc, f)))
            hl = _a_combos(_silu(gt) * up)
            if pend is not None:
                d = pdots(pend[1], d_rhs(pend[0]))
                acc = d if acc is None else [p + t for p, t in zip(acc, d)]
            pend = (f, hl)
        acc = [p + t for p, t in zip(acc, pdots(pend[1], d_rhs(pend[0])))]
        y = _c_full(acc)
        pacer.flush()
        rhs = _rhs7(wo_tile(0, 4, 0, 4), wo_tile(4, 8, 4, 8), lambda k: woc[k])
        s = _c_full([_dot(pltpu.bitcast(ol_s[k], bf16), rhs[k]) for k in range(7)])
        xr = x_v[pl.ds(r_off, SB), :].astype(f32)
        out_v[pl.ds(r_off, SB), :] = (xr + s * _silu(y)).astype(out_v.dtype)
        cp_out(r_off).start()
        return carry

    cp_x(0).start()
    for i in range(NSLAB):
        for cp in cp_q(i):
            cp.start()
    for b in range(NS):
        if b + 1 < NS:
            cp_x(b + 1).start()
        for cp in cp_k(b):
            cp.start()
    for q in range(NQ):
        for cp in cp_v(q) + cp_gu(q):
            cp.start()
    cp_o().start()
    for q in range(NQ):
        for cp in cp_d(q):
            cp.start()
    z_ref[...] = jnp.zeros((8, 128), u32)
    k_s[:, 0:HALO, :] = jnp.zeros((8, HALO, 128), f32)
    v_s[:, 0:HALO, :] = jnp.zeros((8, HALO, 128), f32)
    cp_x(0).wait()
    run_all(ln_stages(0, 0, HB // 16), 3)

    def body_prep(i, carry):
        for cp in cp_q(i):
            cp.wait()
        prep_pair(wq_v, qc_v, pl.multiple_of(i * SLAB, SLAB), SLAB)
        return carry

    lax.fori_loop(0, NSLAB, body_prep, 0)
    lax.fori_loop(0, NS, body_a0, 0)
    lax.fori_loop(0, NQ, body_ak, 0)
    lax.fori_loop(0, NQ, body_av, 0)
    lax.fori_loop(0, NS, body_b, 0)
    for i in range(NS):
        cp_out(i * SB).wait()


def _scratch_shapes():
    vm = pltpu.VMEM
    return [
        vm((S, D), bf16), vm((7, S // 4, DHALF), u32), vm((S, D), bf16),
        vm((D, D), bf16), vm((5, KP, DHALF), u32),
        vm((D, D), bf16), vm((5, KP, DHALF), u32),
        vm((D, D), bf16), vm((5, KP, DHALF), u32),
        vm((D, D), bf16), vm((8, 8 * WOP, 128), u32), vm((5, KP, DHALF), u32),
        vm((D, F), bf16), vm((D, F), bf16), vm((F, D), bf16),
        vm((5, KP, F // 2), u32), vm((5, KP, F // 2), u32), vm((5, F // 4, DHALF), u32),
        vm((8, S, 128), f32), vm((8, HALO + S, 128), f32), vm((8, HALO + S, 128), f32),
        vm((SB, D), f32), vm((7, XP, DHALF), u32), vm((8, 128), u32),
        pltpu.SemaphoreType.DMA((2 + 2 * NS + 2 * NSLAB + 2 * NQ,)),
    ]


@jax.jit
def pallas_recurrent_scan__sliding_local_dilated__swiglu_ffn__prompt_kernel(
    A_x: jax.Array,
    A_wqkv: jax.Array,
    A_wo: jax.Array,
    B_x: jax.Array,
    B_w_gate: jax.Array,
    B_w_up: jax.Array,
    B_w_down: jax.Array,
):
    del B_x
    assert A_x.shape == (1, S, D) and A_wqkv.shape == (D, 3 * D) and B_w_gate.shape == (D, F)
    any_spec = pl.BlockSpec(memory_space=pl.ANY)
    out = pl.pallas_call(
        _kernel,
        in_specs=[any_spec] * 6,
        out_specs=any_spec,
        out_shape=jax.ShapeDtypeStruct((S, D), bf16),
        scratch_shapes=_scratch_shapes(),
        compiler_params=pltpu.CompilerParams(vmem_limit_bytes=124 << 20),
        name="fused_attn_swiglu",
    )(A_x.reshape(S, D), A_wqkv, A_wo, B_w_gate, B_w_up, B_w_down)
    return out.reshape(1, S, D)
```
